```python
import jax
import jax.numpy as jnp

def _softmax(x, axis=-1):
    return jax.nn.softmax(x, axis=axis)

def _gelu(x):
    return jax.nn.gelu(x, approximate=True)

def _silu(x):
    return jax.nn.silu(x)

def _sigmoid(x):
    return jax.nn.sigmoid(x)

def _layernorm(x, axis=-1, eps=1e-05):
    m = jnp.mean(x, axis=axis, keepdims=True)
    v = jnp.var(x, axis=axis, keepdims=True)
    return (x - m) / jnp.sqrt(v + eps)

def _scatter_add(tgt, idx, src, axis=0):
    return tgt.at[idx].add(src)

def _segment_sum(src, seg, n):
    return jax.ops.segment_sum(src, seg, n)

class _Rng:

    def __init__(self, key):
        self._k = key

    def _next(self):
        self._k, sub = jax.random.split(self._k)
        return sub

    def normal(self, shape):
        return jax.random.normal(self._next(), shape, dtype=jnp.bfloat16)

    def randint(self, lo, hi, shape):
        return jax.random.randint(self._next(), shape, lo, hi, dtype=jnp.int32)

    def uniform(self, shape, lo=0.0, hi=1.0):
        return jax.random.uniform(self._next(), shape, jnp.bfloat16, lo, hi)

    def permutation(self, n):
        return jax.random.permutation(self._next(), n)
kernel_name = 'parallel_sum__memory_aug_infini_attn__moe_arch_mod__prompt'

def setup_inputs():
    _rng = _Rng(jax.random.key(int.from_bytes(__import__("os").urandom(4), "little")))
    _w = lambda a: (lambda t: t.astype(jnp.bfloat16) if jnp.issubdtype(t.dtype, jnp.floating) else t)(jnp.asarray(a))

    def _A_setup():
        B, S, D, H = (1, 2048, 576, 32)
        N = 4
        L = max(1, S // N)
        sc = D ** (-0.5)
        return {'x': _w((lambda *s: _rng.normal(s) * 0.05)(B, N * L, D)), 'wq': _w((lambda *s: _rng.normal(s) * 0.05)(D, D) * sc), 'wk': _w((lambda *s: _rng.normal(s) * 0.05)(D, D) * sc), 'wv': _w((lambda *s: _rng.normal(s) * 0.05)(D, D) * sc), 'wo': _w((lambda *s: _rng.normal(s) * 0.05)(D, D) * sc), 'beta': _w((lambda *s: _rng.normal(s) * 0.05)(H))}
    _A_in = _A_setup()

    def _B_setup():
        B, S, D, F, C = (1, 2048, 576, 4608, 2)
        return {'x': _w((lambda *s: _rng.normal(s) * 0.05)(B, S, D)), 'w_r': _w((lambda *s: _rng.normal(s) * 0.05)(D)), 'w_gate': _w((lambda *s: _rng.normal(s) * 0.05)(D, F)), 'w_up': _w((lambda *s: _rng.normal(s) * 0.05)(D, F)), 'w_down': _w((lambda *s: _rng.normal(s) * 0.05)(F, D))}
    _B_in = _B_setup()
    return {'A_x': _A_in['x'], 'A_wq': _A_in['wq'], 'A_wk': _A_in['wk'], 'A_wv': _A_in['wv'], 'A_wo': _A_in['wo'], 'A_beta': _A_in['beta'], 'B_x': _B_in['x'], 'B_w_r': _B_in['w_r'], 'B_w_gate': _B_in['w_gate'], 'B_w_up': _B_in['w_up'], 'B_w_down': _B_in['w_down']}

def reference(A_x, A_wq, A_wk, A_wv, A_wo, A_beta, B_x, B_w_r, B_w_gate, B_w_up, B_w_down):

    def _A_ref(x, wq, wk, wv, wo, beta):
        B, S, D = x.shape
        H = 32
        Dh = D // H
        N = 4
        L = S // N
        q = (lambda x, *d: x.transpose(*d))((x @ wq).reshape(B, S, H, Dh), 0, 2, 1, 3).reshape(B, H, N, L, Dh)
        k = (lambda x, *d: x.transpose(*d))((x @ wk).reshape(B, S, H, Dh), 0, 2, 1, 3).reshape(B, H, N, L, Dh)
        v = (lambda x, *d: x.transpose(*d))((x @ wv).reshape(B, S, H, Dh), 0, 2, 1, 3).reshape(B, H, N, L, Dh)
        phi = lambda t: jnp.where(t > 0, t + 1.0, jnp.exp(t))
        scale = Dh ** (-0.5)
        ar = jnp.arange(L)
        mask = (lambda x, dt: x.astype(dt))(ar[:, None] < ar[None, :], x.dtype) * -1000000000.0
        g = _sigmoid(beta).reshape(1, H, 1, 1)
        M = jnp.einsum('bhd,bhe->bhde', q[:, :, 0, 0, :] * 0.0, q[:, :, 0, 0, :] * 0.0)
        z = q[:, :, 0, 0, :] * 0.0
        outs = []
        for s in range(N):
            qs, ks, vs = (q[:, :, s].copy(), k[:, :, s].copy(), v[:, :, s].copy())
            logits = jnp.einsum('bhqd,bhkd->bhqk', qs, ks) * scale + mask
            p = _softmax(logits, axis=-1)
            a_dot = jnp.einsum('bhqk,bhkd->bhqd', p, vs)
            pq = phi(qs)
            num = jnp.einsum('bhld,bhde->bhle', pq, M)
            den = jnp.einsum('bhld,bhd->bhl', pq, z)[..., None] + 1e-06
            a_mem = num / den
            o = g * a_mem + (1.0 - g) * a_dot
            outs.append(o)
            pk = phi(ks)
            M = M + jnp.einsum('bhld,bhle->bhde', pk, vs)
            z = z + jnp.einsum('bhld->bhd', pk)
        o = (lambda x, *d: x.transpose(*d))(jnp.stack(outs, 2).reshape(B, H, S, Dh), 0, 2, 1, 3).reshape(B, S, D)
        return o @ wo

    def _B_ref(x, w_r, w_gate, w_up, w_down):
        B, S, D = x.shape
        C = 2
        r = x @ w_r
        idx = jnp.argsort(-r, axis=-1)[:, :C]
        idx_e = jnp.repeat(idx.reshape(B, C, 1), D, axis=2)
        x_sel = jnp.take_along_axis(x, idx_e, axis=1)
        g = _silu(x_sel @ w_gate)
        u = x_sel @ w_up
        y = g * u @ w_down
        r_sel = _sigmoid(jnp.take_along_axis(r, idx, axis=1))
        y = y * r_sel.reshape(B, C, 1)
        b_off = (jnp.arange(B) * S).reshape(B, 1)
        flat_idx = (idx + b_off).reshape(B * C)
        zero = (x * 0.0).reshape(B * S, D)
        upd = _scatter_add(zero, flat_idx, y.reshape(B * C, D), axis=0)
        return x + upd.reshape(B, S, D)
    x = A_x
    xn = _layernorm(x, axis=-1)
    return x + _A_ref(xn, A_wq, A_wk, A_wv, A_wo, A_beta) + _B_ref(xn, B_w_r, B_w_gate, B_w_up, B_w_down)
```

```python
import jax
import jax.numpy as jnp
from jax import lax
import jax.experimental.pallas as pl
import jax.experimental.pallas.tpu as pltpu

F32, BF16 = jnp.float32, jnp.bfloat16
S, D, H, DH, NSEG, L, FF = 2048, 576, 32, 18, 4, 512, 4608
T = 128
NT = L // T
HG = 4
GR = HG * DH
GP = 80
NG = H // HG
LOG2E = 1.4426950408889634
QSCALE = DH ** -0.5 * LOG2E
L_LO, L_HI, O_HI = 2.0 ** -40, 2.0 ** 40, 3.0e38
FC = 512
NFC = FF // FC
OC = 144
NT_DIMS = (((1,), (1,)), ((), ()))
V0 = (0, 16, 32, 48)
LROW = (23, 23, 23, 0)


def _iota(shape, dim):
    return lax.broadcasted_iota(jnp.int32, shape, dim)


def _dot(a, b):
    return jnp.dot(a, b, preferred_element_type=F32)


def _dot_nt(a, b):
    return lax.dot_general(a, b, NT_DIMS, preferred_element_type=F32)


def _rb(x):
    return x.astype(BF16).astype(F32)


def _phi(t):
    return jnp.where(t > 0, t + 1.0, jnp.exp(t))


def _pad_bf16(a):
    return jnp.concatenate([a, jnp.zeros((GP - GR, a.shape[1]), F32)], axis=0).astype(BF16)


def _merge_heads(wins):
    a, b, c, e = wins
    r = _iota((8, T), 0)
    return jnp.concatenate(
        [a[0:16], jnp.where(r < 2, a[16:24], b[0:8]), b[8:16],
         jnp.where(r < 4, b[16:24], c[0:8]), c[8:16],
         jnp.where(r < 6, c[16:24], e[0:8]), e[8:24]], axis=0)


def _head_query(q, j):
    lo, hi = DH * j, DH * (j + 1)
    a, b = lo // 16 * 16, min(lo // 16 * 16 + 32, GR)
    r = _iota((b - a, T), 0) + a
    parts = [jnp.where((r >= lo) & (r < hi), q[a:b], 0.0)]
    if a:
        parts = [jnp.zeros((a, T), F32)] + parts
    if b < GP:
        parts = parts + [jnp.zeros((GP - b, T), F32)]
    return jnp.concatenate(parts, axis=0).astype(BF16)


def _head_values(v, j):
    w = v[V0[j]:V0[j] + 24]
    r = _iota((8, v.shape[1]), 0)
    if LROW[j] == 0:
        return jnp.concatenate([jnp.where(r == 0, 1.0, w[0:8]), w[8:24]], axis=0)
    return jnp.concatenate([w[0:16], jnp.where(r == 7, 1.0, w[16:24])], axis=0)


def _kernel(x_hbm, wq_hbm, wk_hbm, wv_hbm, wo_hbm, beta_ref, wr_ref, wg_hbm, wu_hbm, wd_hbm,
            o_hbm, x_v, w_v, wg_v, wu_v, wd_v, xn_s, wt_s, wot_s, ot_s, o_v, y_s, g_s, m_s, sems):
    copies = {}

    def start(key, src, dst):
        copies[key] = pltpu.make_async_copy(src, dst, sems.at[len(copies)])
        copies[key].start()

    def x_copy(s):
        start(("x", s), x_hbm.at[:, pl.ds(s * L, L)], x_v.at[:, pl.ds(s * L, L)])

    x_copy(0)
    for n, w in enumerate((wq_hbm, wk_hbm, wv_hbm)):
        start(("w", n), w, w_v.at[n])
    for s in range(1, NSEG):
        x_copy(s)
    start(("w", 3), wo_hbm, w_v.at[3])
    for c in range(NFC):
        start(("g", c), wg_hbm.at[:, pl.ds(c * FC, FC)], wg_v.at[:, pl.ds(c * FC, FC)])
        start(("u", c), wu_hbm.at[:, pl.ds(c * FC, FC)], wu_v.at[:, pl.ds(c * FC, FC)])
    for c in range(NFC):
        start(("d", c), wd_hbm.at[:, pl.ds(c * FC, FC)], wd_v.at[:, pl.ds(c * FC, FC)])

    def layernorm(t):
        x = x_v[:, t * T:(t + 1) * T].astype(F32)
        m = jnp.sum(x, axis=0, keepdims=True) / D
        d = x - m
        v = _rb(jnp.sum(d * d, axis=0, keepdims=True) / D)
        sd = _rb(jnp.sqrt(_rb(v + _rb(jnp.full((1, T), 1e-5, F32)))))
        xn_s[t] = (_rb(x - _rb(m)) * (1.0 / sd)).astype(BF16)

    def transpose_w(n, c):
        lo, hi = c * T, min((c + 1) * T, D)
        wt = w_v[n, :, lo:hi].astype(F32).T
        if n == 3:
            wot_s[lo:hi] = wt
            return
        for g in range(lo // GR, (hi - 1) // GR + 1):
            a, b = max(lo, g * GR), min(hi, (g + 1) * GR)
            wt_s[g, n * GR + a - g * GR:n * GR + b - g * GR] = wt[a - lo:b - lo]

    def seg_xn(s):
        return jnp.concatenate([xn_s[s * NT + i] for i in range(NT)], axis=1)

    def project(s, g):
        r = _dot(wt_s[g], seg_xn(s))
        q, k, v = r[0:GR], r[GR:2 * GR], r[2 * GR:3 * GR]
        return dict(q=q, k=k, v=v, kn=_pad_bf16(k).T)

    def mem_mask():
        r, c = _iota((GP, GP), 0), _iota((GP, GP), 1)
        keep = None
        for j in range(HG):
            rows = ((r >= DH * j) & (r < DH * (j + 1))) | (r == GR + j)
            blk = rows & (c >= DH * j) & (c < DH * (j + 1))
            keep = blk if keep is None else keep | blk
        return keep

    def mem_delta(u):
        pk = _pad_bf16(_phi(u["k"]))
        lhs = jnp.concatenate([u["v"], jnp.ones((GP - GR, L), F32)], axis=0)
        acc = None
        for i in range(NT):
            part = _dot_nt(lhs[:, i * T:(i + 1) * T], pk[:, i * T:(i + 1) * T])
            acc = part if acc is None else acc + part
        return jnp.where(mem_mask(), acc, 0.0)

    def mem_read(u, mem, gate):
        r = _dot(mem, _pad_bf16(_phi(u["q"])))
        coef = gate / (r[GR:GP] + 1e-6)
        out = []
        for i in range(NT):
            ci = coef[:, i * T:(i + 1) * T]
            wins = [jnp.broadcast_to(ci[j:j + 1], (24, T)) for j in range(HG)]
            out.append(r[0:GR, i * T:(i + 1) * T] * _merge_heads(wins))
        return out

    def gate_rows(g):
        return g_s[g]

    def finish(accs, gate, mem_i):
        dens = [accs[j][LROW[j]:LROW[j] + 1] for j in range(HG)]
        o = _merge_heads([accs[j] * ((1.0 - gate[j:j + 1]) / dens[j]) for j in range(HG)])
        return (o if mem_i is None else o + mem_i), dens

    def out_rows(s, c, idx):
        rows = pl.ds(c * OC, OC)
        cols = pl.ds(s * L if isinstance(s, int) else pl.multiple_of(s * L, L), L)
        a = _dot(wot_s[rows], ot_s[s].astype(BF16))
        tok = _iota((1, L), 1) + s * L
        y0, y1 = (jnp.concatenate([y_s[n, rows]] * NT, axis=1) for n in range(2))
        upd = jnp.where(tok == idx[0], y0, jnp.where(tok == idx[1], y1, 0.0))
        xn = jnp.concatenate([xn_s[s * NT + i, rows] for i in range(NT)], axis=1)
        o_v[rows, cols] = ((x_v[rows, cols].astype(F32) + a) + (xn.astype(F32) + upd)).astype(BF16)

    st = {}

    def gates():
        sg = jax.nn.sigmoid(beta_ref[...].astype(F32).reshape(1, H))
        for g in range(NG):
            pick = _iota((8, H), 1) == _iota((8, H), 0) + HG * g
            col = jnp.sum(jnp.where(pick, sg, 0.0), axis=1, keepdims=True)
            g_s[g] = jnp.broadcast_to(col, (8, T))

    def router(s):
        wr = jnp.broadcast_to(wr_ref[...].astype(F32).reshape(1, D), (8, D))
        st["r", s] = _rb(_dot(wr, seg_xn(s)))

    def top2():
        r = jnp.concatenate([st["r", s][0:1] for s in range(NSEG)], axis=1)
        tok = _iota((1, S), 1)
        idx, val, sel = [], [], None
        for n in range(2):
            best = jnp.max(r, axis=1, keepdims=True)
            i = jnp.clip(jnp.min(jnp.where(r == best, tok, S)), 0, S - 1)
            r = jnp.where(tok == i, -jnp.inf, r)
            hot = ((_iota((8, T), 1) == i % T) & (_iota((8, T), 0) == n)).astype(F32)
            row = _dot_nt(hot, xn_s[i // T])
            sel = row if sel is None else sel + row
            idx.append(i)
            val.append(best)
        st["idx"], st["xs"] = idx, sel
        st["rs"] = jax.nn.sigmoid(jnp.where(_iota((8, 1), 0) == 0, val[0], val[1]))

    def ffn_in(name, w, c, kt):
        lo, hi = kt * T, min((kt + 1) * T, D)
        part = _dot(st["xs"][:, lo:hi], w[lo:hi, c * FC:(c + 1) * FC])
        st[name, c] = part if kt == 0 else st[name, c] + part

    def ffn_act(c):
        g = st.pop(("g", c))
        st["h", c] = g * jax.nn.sigmoid(g) * st.pop(("u", c))

    def ffn_out(c, ft, lo, hi):
        f = c * FC + ft * T
        part = _dot_nt(st["h", c][:, ft * T:(ft + 1) * T], wd_v[lo:hi, f:f + T])
        st["y", lo] = part if (c, ft) == (0, 0) else st["y", lo] + part

    def ffn_finish():
        y = jnp.concatenate([st["y", 0], st["y", 512]], axis=1) * st["rs"]
        for n in range(2):
            y_s[n] = jnp.broadcast_to(y[n:n + 1], (T, D)).T

    units, mems = {}, {}
    tiles = [(u, i, c) for u in range(NSEG * NG) for i in (3, 2, 1, 0) for c in range(i + 1)]
    per_unit = NT * (NT + 1) // 2
    tri = _iota((T, T), 0) <= _iota((T, T), 1)
    rng = dict(lo=jnp.ones((1, T), F32), hi=jnp.ones((1, T), F32), o=jnp.zeros((8, T), F32))

    def do_project(u):
        units[u] = project(u // NG, u % NG)

    def do_mem_read(u):
        gate = jnp.concatenate([gate_rows(u % NG)] * NT, axis=1)
        units[u]["mem"] = mem_read(units[u], mems[u % NG], gate)

    def do_mem_update(u):
        delta = mem_delta(units[u])
        mems[u % NG] = delta if u < NG else mems[u % NG] + delta

    def scores(t):
        u, i, c = tiles[t]
        un = units[u]
        if c == 0:
            q = un["q"][:, i * T:(i + 1) * T] * QSCALE
            un["qm"] = jnp.concatenate([_head_query(q, j) for j in range(HG)], axis=1)
        s = _dot(un["kn"][c * T:(c + 1) * T], un["qm"])
        ps = []
        for j in range(HG):
            p = jnp.exp2(s[:, j * T:(j + 1) * T])
            ps.append((jnp.where(tri, p, 0.0) if c == i else p).astype(BF16))
        st["p", t] = ps

    def values(t):
        u, i, c = tiles[t]
        un = units[u]
        ps = st.pop(("p", t))
        v = un["v"][:, c * T:(c + 1) * T]
        for j in range(HG):
            part = _dot(_head_values(v, j), ps[j])
            st["o", j] = part if c == 0 else st["o", j] + part
        if c == i:
            mem_i = un["mem"][i] if "mem" in un else None
            o, dens = finish([st["o", j] for j in range(HG)], gate_rows(u % NG), mem_i)
            ot_s[u // NG, (u % NG) * GR:(u % NG + 1) * GR, i * T:(i + 1) * T] = o
            for l in dens:
                rng["lo"], rng["hi"] = jnp.minimum(rng["lo"], l), jnp.maximum(rng["hi"], l)
            rng["o"] = jnp.maximum(rng["o"], jnp.max(jnp.abs(o).reshape(GR // 8, 8, T), axis=0))

    def do_out(s, c):
        out_rows(s, c, st["idx"])
        rows, cols = pl.ds(c * OC, OC), pl.ds(s * L, L)
        start(("o", s, c), o_v.at[rows, cols], o_hbm.at[rows, cols])

    fill = {}

    def at(step, fn, *args):
        fill.setdefault(step, []).append((fn, args))

    def wait(key):
        copies[key].wait()

    nu = NSEG * NG
    for u in range(nu):
        t0 = u * per_unit
        if u + 1 < nu:
            at(t0 + 3, do_project, u + 1)
        if u >= NG:
            at(t0 + 1, do_mem_read, u)
        if u < nu - NG:
            at(t0 + 7, do_mem_update, u)
    for c in range(1, 5):
        for n in range(3):
            at(max((T * c // GR - 1) * per_unit, 0) + n, transpose_w, n, c)
    for s in range(1, NSEG):
        at(s * per_unit + 4, wait, ("x", s))
        for i in range(NT):
            at(s * per_unit + 4 + i, layernorm, s * NT + i)
    for s in range(NSEG):
        at(4 * per_unit + s, router, s)
    at(4 * per_unit + 6, top2)
    at(7 * per_unit, wait, ("w", 3))
    for c in range(5):
        at(7 * per_unit + c, transpose_w, 3, c)
    step = 5 * per_unit
    for c in range(NFC):
        for name, w in (("g", wg_v), ("u", wu_v)):
            at(step, wait, (name, c))
            for kt in range(5):
                at(step, ffn_in, name, w, c, kt)
                step += 1
        at(step + 1, ffn_act, c)
    step += 2
    for c in range(NFC):
        at(step, wait, ("d", c))
        for ft in range(FC // T):
            at(step, ffn_out, c, ft, 0, 512)
            at(step, ffn_out, c, ft, 512, D)
            step += 1
    at(step + 1, ffn_finish)
    first = step // per_unit + 2
    chunks = [(s, c) for s in range(NSEG - 1) for c in range(D // OC)]
    for n, (s, c) in enumerate(chunks[:-1]):
        at((first + n) * per_unit + 5, do_out, s, c)

    gates()
    wait(("x", 0))
    for i in range(NT):
        layernorm(i)
    for n in range(3):
        wait(("w", n))
        transpose_w(n, 0)
    do_project(0)
    lag = 2
    for t in range(len(tiles) + lag):
        for fn, args in fill.pop(t, []):
            fn(*args)
        if t < len(tiles):
            scores(t)
        if t == len(tiles):
            do_out(*chunks[-1])
        if t >= lag:
            values(t - lag)
    assert not fill
    for c in range(D // OC):
        do_out(NSEG - 1, c)
    for key in copies:
        if key[0] == "o":
            wait(key)

    safe = (jnp.min(rng["lo"]) >= L_LO) & (jnp.max(rng["hi"]) <= L_HI) & (jnp.max(rng["o"]) <= O_HI)

    @pl.when(jnp.logical_not(safe))
    def _():
        m_s[...] = jnp.zeros(m_s.shape, F32)

        def unit(u, carry):
            s, g = u // NG, u % NG
            un = project(s, g)
            gate = gate_rows(g)
            mem = mem_read(un, m_s[g], jnp.concatenate([gate] * NT, axis=1))
            for i in range(NT):
                nk = (i + 1) * T
                q = un["q"][:, i * T:nk] * QSCALE
                keep = _iota((nk, T), 0) <= _iota((nk, T), 1) + i * T
                accs = []
                for j in range(HG):
                    sc = jnp.where(keep, _dot(un["kn"][0:nk], _head_query(q, j)), -jnp.inf)
                    p = jnp.exp2(sc - jnp.max(sc, axis=0, keepdims=True))
                    accs.append(_dot(_head_values(un["v"][:, 0:nk], j), p.astype(BF16)))
                o, _ = finish(accs, gate, mem[i])
                ot_s[s, pl.ds(pl.multiple_of(g * GR, 8), GR), i * T:nk] = o
            m_s[g] += mem_delta(un)
            return carry

        lax.fori_loop(0, nu, unit, 0)

        def segment(s, carry):
            for c in range(D // OC):
                out_rows(s, c, st["idx"])
            return carry

        lax.fori_loop(0, NSEG, segment, 0)
        redo = pltpu.make_async_copy(o_v, o_hbm, sems.at[0])
        redo.start()
        redo.wait()


@jax.jit
def pallas_parallel_sum__memory_aug_infini_attn__moe_arch_mod__prompt_kernel(
    A_x: jax.Array,
    A_wq: jax.Array,
    A_wk: jax.Array,
    A_wv: jax.Array,
    A_wo: jax.Array,
    A_beta: jax.Array,
    B_x: jax.Array,
    B_w_r: jax.Array,
    B_w_gate: jax.Array,
    B_w_up: jax.Array,
    B_w_down: jax.Array,
):
    del B_x
    hbm = pl.BlockSpec(memory_space=pltpu.HBM)
    vmem = pl.BlockSpec(memory_space=pltpu.VMEM)
    nsem = NSEG + 4 + 3 * NFC + NSEG * (D // OC)
    out = pl.pallas_call(
        _kernel,
        out_shape=jax.ShapeDtypeStruct((D, S), BF16),
        in_specs=[hbm] * 5 + [vmem] * 2 + [hbm] * 3,
        out_specs=hbm,
        scratch_shapes=[
            pltpu.VMEM((D, S), BF16),
            pltpu.VMEM((4, D, D), BF16),
            pltpu.VMEM((D, FF), BF16),
            pltpu.VMEM((D, FF), BF16),
            pltpu.VMEM((D, FF), BF16),
            pltpu.VMEM((S // T, D, T), BF16),
            pltpu.VMEM((NG, 3 * GR, D), F32),
            pltpu.VMEM((D, D), F32),
            pltpu.VMEM((NSEG, D, L), F32),
            pltpu.VMEM((D, S), BF16),
            pltpu.VMEM((2, D, T), F32),
            pltpu.VMEM((NG, 8, T), F32),
            pltpu.VMEM((NG, GP, GP), F32),
            pltpu.SemaphoreType.DMA((nsem,)),
        ],
        compiler_params=pltpu.CompilerParams(vmem_limit_bytes=100 * 1024 * 1024),
        name="infini_mod",
    )(A_x.reshape(S, D).T, A_wq, A_wk, A_wv, A_wo, A_beta, B_w_r, B_w_gate, B_w_up, B_w_down.T)
    return out.T.reshape(1, S, D)
```

```python
import jax
import jax.numpy as jnp
from jax import lax
import jax.experimental.pallas as pl
import jax.experimental.pallas.tpu as pltpu

F32, BF16 = jnp.float32, jnp.bfloat16
S, D, H, DH, NSEG, L, FF = 2048, 576, 32, 18, 4, 512, 4608
T = 128
NT = L // T
HG = 4
GR = HG * DH
GP = 80
NG = H // HG
LOG2E = 1.4426950408889634
QSCALE = DH ** -0.5 * LOG2E
L_LO, L_HI, O_HI = 2.0 ** -40, 2.0 ** 40, 3.0e38
FC = 512
NFC = FF // FC
OC = 144
NT_DIMS = (((1,), (1,)), ((), ()))
V0 = (0, 16, 32, 48)
LROW = (23, 23, 23, 0)


def _iota(shape, dim):
    return lax.broadcasted_iota(jnp.int32, shape, dim)


def _dot(a, b):
    return jnp.dot(a, b, preferred_element_type=F32)


def _dot_nt(a, b):
    return lax.dot_general(a, b, NT_DIMS, preferred_element_type=F32)


def _rb(x):
    return x.astype(BF16).astype(F32)


def _phi(t):
    return jnp.where(t > 0, t + 1.0, jnp.exp(t))


def _pad_bf16(a):
    return jnp.concatenate([a, jnp.zeros((GP - GR, a.shape[1]), F32)], axis=0).astype(BF16)


def _merge_heads(wins):
    a, b, c, e = wins
    r = _iota((8, T), 0)
    return jnp.concatenate(
        [a[0:16], jnp.where(r < 2, a[16:24], b[0:8]), b[8:16],
         jnp.where(r < 4, b[16:24], c[0:8]), c[8:16],
         jnp.where(r < 6, c[16:24], e[0:8]), e[8:24]], axis=0)


def _head_query(q, j):
    lo, hi = DH * j, DH * (j + 1)
    a, b = lo // 16 * 16, min(lo // 16 * 16 + 32, GR)
    r = _iota((b - a, T), 0) + a
    parts = [jnp.where((r >= lo) & (r < hi), q[a:b], 0.0)]
    if a:
        parts = [jnp.zeros((a, T), F32)] + parts
    if b < GP:
        parts = parts + [jnp.zeros((GP - b, T), F32)]
    return jnp.concatenate(parts, axis=0).astype(BF16)


def _head_values(v, j, one=1.0):
    w = v[V0[j]:V0[j] + 24]
    r = _iota((8, v.shape[1]), 0)
    if LROW[j] == 0:
        return jnp.concatenate([jnp.where(r == 0, one, w[0:8]), w[8:24]], axis=0)
    return jnp.concatenate([w[0:16], jnp.where(r == 7, one, w[16:24])], axis=0)


def _kernel(x_hbm, wq_hbm, wk_hbm, wv_hbm, wo_hbm, beta_ref, wr_ref, wg_hbm, wu_hbm, wd_hbm,
            o_hbm, x_v, w_v, wg_v, wu_v, wd_v, xn_s, wt_s, wot_s, ot_s, o_v, y_s, g_s, m_s, sems):
    copies = {}

    def start(key, src, dst):
        copies[key] = pltpu.make_async_copy(src, dst, sems.at[len(copies)])
        copies[key].start()

    def wait(*keys):
        for key in keys:
            copies[key].wait()

    def x_cols(key, lo, hi):
        start(key, x_hbm.at[:, pl.ds(lo, hi - lo)], x_v.at[:, pl.ds(lo, hi - lo)])

    def w_cols(key, lo, hi):
        for n, w in enumerate((wq_hbm, wk_hbm, wv_hbm)):
            start((key, n), w.at[:, pl.ds(lo, hi - lo)], w_v.at[n, :, pl.ds(lo, hi - lo)])

    x_cols("xa", 0, L // 2)
    w_cols("wa", 0, T)
    x_cols("xb", L // 2, L)
    w_cols("wb", T, D)
    x_cols("xc", L, S)
    start("wo", wo_hbm, w_v.at[3])
    start("g", wg_hbm, wg_v)
    start("u", wu_hbm, wu_v)
    start("d", wd_hbm, wd_v)

    st = {}

    def layernorm(t):
        x = x_v[:, t * T:(t + 1) * T].astype(F32)
        m = jnp.sum(x, axis=0, keepdims=True) / D
        d = x - m
        v = _rb(jnp.sum(d * d, axis=0, keepdims=True) / D)
        sd = _rb(jnp.sqrt(_rb(v + _rb(jnp.full((1, T), 1e-5, F32)))))
        xn = (_rb(x - _rb(m)) * (1.0 / sd)).astype(BF16)
        xn_s[t] = xn
        st["r", t] = _rb(jnp.sum(xn.astype(F32) * st["wr"], axis=0, keepdims=True))

    def transpose_w(n, c):
        lo, hi = c * T, min((c + 1) * T, D)
        wt = w_v[n, :, lo:hi].astype(F32).T
        if n == 3:
            wot_s[lo:hi] = wt
            return
        for g in range(lo // GR, (hi - 1) // GR + 1):
            a, b = max(lo, g * GR), min(hi, (g + 1) * GR)
            wt_s[g, n * GR + a - g * GR:n * GR + b - g * GR] = wt[a - lo:b - lo]

    def seg_xn(s):
        return jnp.concatenate([xn_s[s * NT + i] for i in range(NT)], axis=1)

    def project(s, g):
        r = _dot(wt_s[g], seg_xn(s))
        q, k, v = r[0:GR], r[GR:2 * GR], r[2 * GR:3 * GR]
        return dict(q=q, k=k, v=v, kn=_pad_bf16(k).T)

    def mem_mask():
        r, c = _iota((GP, GP), 0), _iota((GP, GP), 1)
        keep = None
        for j in range(HG):
            rows = ((r >= DH * j) & (r < DH * (j + 1))) | (r == GR + j)
            blk = rows & (c >= DH * j) & (c < DH * (j + 1))
            keep = blk if keep is None else keep | blk
        return keep

    def mem_delta(u):
        pk = _pad_bf16(_phi(u["k"]))
        lhs = jnp.concatenate([u["v"], jnp.ones((GP - GR, L), F32)], axis=0)
        acc = None
        for i in range(NT):
            part = _dot_nt(lhs[:, i * T:(i + 1) * T], pk[:, i * T:(i + 1) * T])
            acc = part if acc is None else acc + part
        return jnp.where(mem_mask(), acc, 0.0)

    def mem_read(u, mem, gate):
        r = _dot(mem, _pad_bf16(_phi(u["q"])))
        coef = gate / (r[GR:GP] + 1e-6)
        out = []
        for i in range(NT):
            ci = coef[:, i * T:(i + 1) * T]
            wins = [jnp.broadcast_to(ci[j:j + 1], (24, T)) for j in range(HG)]
            out.append(r[0:GR, i * T:(i + 1) * T] * _merge_heads(wins))
        return out

    def gate_rows(g):
        return g_s[g]

    def finish(accs, gate, mem_i):
        dens = [accs[j][LROW[j]:LROW[j] + 1] for j in range(HG)]
        o = _merge_heads([accs[j] * ((1.0 - gate[j:j + 1]) / dens[j]) for j in range(HG)])
        return (o if mem_i is None else o + mem_i), dens

    def out_rows(s, c, idx):
        rows = pl.ds(c * OC, OC)
        cols = pl.ds(s * L if isinstance(s, int) else pl.multiple_of(s * L, L), L)
        a = _dot(wot_s[rows], ot_s[s].astype(BF16))
        tok = _iota((1, L), 1) + s * L
        y0, y1 = (jnp.concatenate([y_s[n, rows]] * NT, axis=1) for n in range(2))
        upd = jnp.where(tok == idx[0], y0, jnp.where(tok == idx[1], y1, 0.0))
        xn = jnp.concatenate([xn_s[s * NT + i, rows] for i in range(NT)], axis=1)
        o_v[rows, cols] = ((x_v[rows, cols].astype(F32) + a) + (xn.astype(F32) + upd)).astype(BF16)

    def gates():
        sg = jax.nn.sigmoid(beta_ref[...].astype(F32).reshape(1, H))
        for g in range(NG):
            pick = _iota((8, H), 1) == _iota((8, H), 0) + HG * g
            col = jnp.sum(jnp.where(pick, sg, 0.0), axis=1, keepdims=True)
            g_s[g] = jnp.broadcast_to(col, (8, T))

    def pick(n):
        if n == 0:
            st["r"] = jnp.concatenate([st["r", t] for t in range(S // T)], axis=1)
            st["idx"], st["val"] = [], []
        tok = _iota((1, S), 1)
        best = jnp.max(st["r"], axis=1, keepdims=True)
        i = jnp.clip(jnp.min(jnp.where(st["r"] == best, tok, S)), 0, S - 1)
        st["r"] = jnp.where(tok == i, -jnp.inf, st["r"])
        st["idx"].append(i)
        st["val"].append(best)

    def gather(n):
        i = st["idx"][n]
        hot = ((_iota((8, T), 1) == i % T) & (_iota((8, T), 0) == n)).astype(F32)
        row = _dot_nt(hot, xn_s[i // T])
        st["xs"] = row if n == 0 else st["xs"] + row

    def ffn_in(name, w, c, kt):
        lo, hi = kt * T, min((kt + 1) * T, D)
        part = _dot(st["xs"][:, lo:hi], w[lo:hi, c * FC:(c + 1) * FC])
        st[name, c] = part if kt == 0 else st[name, c] + part

    def ffn_act(c):
        g = st.pop(("g", c))
        st["h", c] = g * jax.nn.sigmoid(g) * st.pop(("u", c))

    def ffn_out(c, ft, lo, hi):
        f = c * FC + ft * T
        part = _dot_nt(st["h", c][:, ft * T:(ft + 1) * T], wd_v[lo:hi, f:f + T])
        st["y", lo] = part if (c, ft) == (0, 0) else st["y", lo] + part

    def ffn_finish():
        gate = jax.nn.sigmoid(jnp.where(_iota((8, 1), 0) == 0, *st["val"]))
        y = jnp.concatenate([st["y", 0], st["y", 512]], axis=1) * gate
        for n in range(2):
            y_s[n] = jnp.broadcast_to(y[n:n + 1], (T, D)).T

    units, mems = {}, {}
    tiles = [(u, i, c) for u in range(NSEG * NG) for i in (3, 2, 1, 0) for c in range(i + 1)]
    per_unit = NT * (NT + 1) // 2
    tri = _iota((T, T), 0) <= _iota((T, T), 1)
    rng = dict(lo=jnp.ones((1, T), F32), hi=jnp.ones((1, T), F32), o=jnp.zeros((8, T), F32))

    def do_project(u):
        units[u] = project(u // NG, u % NG)

    def do_mem_read(u):
        gate = jnp.concatenate([gate_rows(u % NG)] * NT, axis=1)
        units[u]["mem"] = mem_read(units[u], mems[u % NG], gate)

    def do_mem_update(u):
        delta = mem_delta(units[u])
        mems[u % NG] = delta if u < NG else mems[u % NG] + delta

    def scores(t):
        u, i, c = tiles[t]
        un = units[u]
        if c == 0:
            q = un["q"][:, i * T:(i + 1) * T] * QSCALE
            un["qm"] = jnp.concatenate([_head_query(q, j) for j in range(HG)], axis=1)
        s = _dot(un["kn"][c * T:(c + 1) * T], un["qm"])
        ps = []
        for j in range(HG):
            p = jnp.exp2(s[:, j * T:(j + 1) * T])
            ps.append((jnp.where(tri, p, 0.0) if c == i else p).astype(BF16))
        st["p", t] = ps

    def values(t):
        u, i, c = tiles[t]
        un = units[u]
        ps = st.pop(("p", t))
        v = un["v"][:, c * T:(c + 1) * T]
        one = 1.0
        for a in st.pop("due", []):
            one = jnp.maximum(jnp.minimum(a, one), one)
        for j in range(HG):
            part = _dot(_head_values(v, j, one), ps[j])
            st["o", j] = part if c == 0 else st["o", j] + part
        if c == i:
            mem_i = un["mem"][i] if "mem" in un else None
            o, dens = finish([st["o", j] for j in range(HG)], gate_rows(u % NG), mem_i)
            ot_s[u // NG, (u % NG) * GR:(u % NG + 1) * GR, i * T:(i + 1) * T] = o
            for l in dens:
                rng["lo"], rng["hi"] = jnp.minimum(rng["lo"], l), jnp.maximum(rng["hi"], l)
            rng["o"] = jnp.maximum(rng["o"], jnp.max(jnp.abs(o).reshape(GR // 8, 8, T), axis=0))

    def due(*keys):
        st.setdefault("due", []).append(st[keys])

    def do_out(s, c):
        out_rows(s, c, st["idx"])
        rows, cols = pl.ds(c * OC, OC), pl.ds(s * L, L)
        start(("o", s, c), o_v.at[rows, cols], o_hbm.at[rows, cols])

    fill = {}

    def at(step, fn, *args):
        fill.setdefault(step, []).append((fn, args))

    nu = NSEG * NG
    for u in range(nu):
        t0 = u * per_unit
        if u + 1 < nu:
            at(t0 + (3 if u else 5), do_project, u + 1)
        if u >= NG:
            at(t0 + 1, do_mem_read, u)
        if u < nu - NG:
            at(t0 + 7, do_mem_update, u)
    at(2, wait, ("wb", 0), ("wb", 1), ("wb", 2))
    for c in range(1, 5):
        for n in range(3):
            at(max((T * c // GR - 1) * per_unit, 2), transpose_w, n, c)
    at(2 * per_unit + 4, wait, "xc", "wo")
    for t in range(NT, S // T):
        at(2 * per_unit + 4, layernorm, t)
        at(3 * per_unit + 3 + (t - NT) * 5, due, "r", t)
    for n in range(2):
        at((9 + n) * per_unit + 6, pick, n)
        at((11 + n) * per_unit + 4, gather, n)
    for c in range(5):
        at((8 + c) * per_unit + 8, transpose_w, 3, c)
    step = 15 * per_unit + 4
    at(step, wait, "g", "u")
    for c in range(NFC):
        for name, w in (("g", wg_v), ("u", wu_v)):
            for kt in range(5):
                at(step, ffn_in, name, w, c, kt)
                step += 1
        at(step + 1, ffn_act, c)
    step += 2
    at(step, wait, "d")
    for c in range(NFC):
        for ft in range(FC // T):
            at(step, ffn_out, c, ft, 0, 512)
            at(step, ffn_out, c, ft, 512, D)
            step += 1
    at(step + 1, ffn_finish)
    chunks = [(s, c) for s in range(NSEG - 1) for c in range(D // OC)]
    gap = (len(tiles) - step - 6) // (len(chunks) - 1)
    for n, (s, c) in enumerate(chunks[:-1]):
        at(step + 6 + n * gap, do_out, s, c)

    gates()
    st["wr"] = jnp.broadcast_to(wr_ref[...].astype(F32).reshape(1, D), (T, D)).T
    wait("xa")
    layernorm(0)
    layernorm(1)
    wait(("wa", 0), ("wa", 1), ("wa", 2))
    for n in range(3):
        transpose_w(n, 0)
    wait("xb")
    layernorm(2)
    layernorm(3)
    do_project(0)
    lag = 2
    for t in range(len(tiles) + lag):
        for fn, args in fill.pop(t, []):
            fn(*args)
        if t < len(tiles):
            scores(t)
        if t == len(tiles):
            do_out(*chunks[-1])
        if t >= lag:
            values(t - lag)
    assert not fill
    for c in range(D // OC):
        do_out(NSEG - 1, c)
    safe = (jnp.min(rng["lo"]) >= L_LO) & (jnp.max(rng["hi"]) <= L_HI) & (jnp.max(rng["o"]) <= O_HI)
    wait(*[key for key in copies if key[0] == "o" and key != "o"])

    @pl.when(jnp.logical_not(safe))
    def _():
        m_s[...] = jnp.zeros(m_s.shape, F32)

        def unit(u, carry):
            s, g = u // NG, u % NG
            un = project(s, g)
            gate = gate_rows(g)
            mem = mem_read(un, m_s[g], jnp.concatenate([gate] * NT, axis=1))
            for i in range(NT):
                nk = (i + 1) * T
                q = un["q"][:, i * T:nk] * QSCALE
                keep = _iota((nk, T), 0) <= _iota((nk, T), 1) + i * T
                accs = []
                for j in range(HG):
                    sc = jnp.where(keep, _dot(un["kn"][0:nk], _head_query(q, j)), -jnp.inf)
                    p = jnp.exp2(sc - jnp.max(sc, axis=0, keepdims=True))
                    accs.append(_dot(_head_values(un["v"][:, 0:nk], j), p.astype(BF16)))
                o, _ = finish(accs, gate, mem[i])
                ot_s[s, pl.ds(pl.multiple_of(g * GR, 8), GR), i * T:nk] = o
            m_s[g] += mem_delta(un)
            return carry

        lax.fori_loop(0, nu, unit, 0)

        def segment(s, carry):
            for c in range(D // OC):
                out_rows(s, c, st["idx"])
            return carry

        lax.fori_loop(0, NSEG, segment, 0)
        redo = pltpu.make_async_copy(o_v, o_hbm, sems.at[0])
        redo.start()
        redo.wait()


@jax.jit
def pallas_parallel_sum__memory_aug_infini_attn__moe_arch_mod__prompt_kernel(
    A_x: jax.Array,
    A_wq: jax.Array,
    A_wk: jax.Array,
    A_wv: jax.Array,
    A_wo: jax.Array,
    A_beta: jax.Array,
    B_x: jax.Array,
    B_w_r: jax.Array,
    B_w_gate: jax.Array,
    B_w_up: jax.Array,
    B_w_down: jax.Array,
):
    del B_x
    hbm = pl.BlockSpec(memory_space=pltpu.HBM)
    vmem = pl.BlockSpec(memory_space=pltpu.VMEM)
    nsem = 13 + NSEG * (D // OC)
    out = pl.pallas_call(
        _kernel,
        out_shape=jax.ShapeDtypeStruct((D, S), BF16),
        in_specs=[hbm] * 5 + [vmem] * 2 + [hbm] * 3,
        out_specs=hbm,
        scratch_shapes=[
            pltpu.VMEM((D, S), BF16),
            pltpu.VMEM((4, D, D), BF16),
            pltpu.VMEM((D, FF), BF16),
            pltpu.VMEM((D, FF), BF16),
            pltpu.VMEM((D, FF), BF16),
            pltpu.VMEM((S // T, D, T), BF16),
            pltpu.VMEM((NG, 3 * GR, D), F32),
            pltpu.VMEM((D, D), F32),
            pltpu.VMEM((NSEG, D, L), F32),
            pltpu.VMEM((D, S), BF16),
            pltpu.VMEM((2, D, T), F32),
            pltpu.VMEM((NG, 8, T), F32),
            pltpu.VMEM((NG, GP, GP), F32),
            pltpu.SemaphoreType.DMA((nsem,)),
        ],
        compiler_params=pltpu.CompilerParams(vmem_limit_bytes=100 * 1024 * 1024),
        name="infini_mod",
    )(A_x.reshape(S, D).T, A_wq, A_wk, A_wv, A_wo, A_beta, B_w_r, B_w_gate, B_w_up, B_w_down.T)
    return out.T.reshape(1, S, D)
```

```python
import jax
import jax.numpy as jnp
from jax import lax
import jax.experimental.pallas as pl
import jax.experimental.pallas.tpu as pltpu

F32, BF16 = jnp.float32, jnp.bfloat16
S, D, H, DH, NSEG, L, FF = 2048, 576, 32, 18, 4, 512, 4608
T = 128
QB = T // 4
NT = L // T
HG = 4
GR = HG * DH
GP = 80
NG = H // HG
LOG2E = 1.4426950408889634
QSCALE = DH ** -0.5 * LOG2E
L_LO, L_HI, O_HI = 2.0 ** -40, 2.0 ** 40, 3.0e38
FC = 512
OC = 144
NT_DIMS = (((1,), (1,)), ((), ()))
V0 = (0, 16, 32, 48)
LROW = (23, 23, 23, 0)
CFG = dict(order=(2, 0, 3, 1), lag=2, proj=3, read=1, upd=7, merge=1, ffn0=16, wstep=7, odue=2, gstep=6, r0=4, l0=5, ls=5, ys=1.0, s1=2, s2=-3)


def _iota(shape, dim):
    return lax.broadcasted_iota(jnp.int32, shape, dim)


def _dot(a, b):
    return jnp.dot(a, b, preferred_element_type=F32)


def _dot_nt(a, b):
    return lax.dot_general(a, b, NT_DIMS, preferred_element_type=F32)


def _rb(x):
    return x.astype(BF16).astype(F32)


def _colsum(x, chains=1):
    n = x.shape[0] // chains
    p = [jnp.sum(x[i * n:(i + 1) * n].reshape(n // 8, 8, x.shape[1]), axis=0) for i in range(chains)]
    return jnp.sum(sum(p[1:], p[0]), axis=0, keepdims=True)


def _phi(t):
    return jnp.where(t > 0, t + 1.0, jnp.exp(t))


def _pad_bf16(a):
    return jnp.concatenate([a, jnp.zeros((GP - GR, a.shape[1]), F32)], axis=0).astype(BF16)


def _merge_heads(wins):
    a, b, c, e = wins
    r = _iota((8, T), 0)
    return jnp.concatenate(
        [a[0:16], jnp.where(r < 2, a[16:24], b[0:8]), b[8:16],
         jnp.where(r < 4, b[16:24], c[0:8]), c[8:16],
         jnp.where(r < 6, c[16:24], e[0:8]), e[8:24]], axis=0)


def _rotate(a, quarters):
    return pltpu.roll(a, quarters % 4 * QB, 1) if quarters % 4 else a


def _head_query(q, j):
    lo, hi = DH * j, DH * (j + 1)
    a, b = lo // 16 * 16, min(lo // 16 * 16 + 32, GR)
    r = _iota((b - a, T), 0) + a
    parts = [jnp.where((r >= lo) & (r < hi), q[a:b], 0.0)]
    if a:
        parts = [jnp.zeros((a, T), F32)] + parts
    if b < GP:
        parts = parts + [jnp.zeros((GP - b, T), F32)]
    return jnp.concatenate(parts, axis=0).astype(BF16)


def _head_values(v, j, one=1.0):
    w = v[V0[j]:V0[j] + 24]
    r = _iota((8, v.shape[1]), 0)
    if LROW[j] == 0:
        return jnp.concatenate([jnp.where(r == 0, one, w[0:8]), w[8:24]], axis=0)
    return jnp.concatenate([w[0:16], jnp.where(r == 7, one, w[16:24])], axis=0)


def _kernel(x_hbm, wq_hbm, wk_hbm, wv_hbm, wo_hbm, beta_hbm, wr_hbm, wg_hbm, wu_hbm, wd_hbm,
            o_hbm, beta_ref, wr_ref, x_v, w_v, wg_v, wu_v, wd_v, xn_s, wt_s, wot_s, ot_s, o_v, h_s, y_s, g_s, m_s, sems):
    copies = {}

    def start(key, src, dst):
        copies[key] = pltpu.make_async_copy(src, dst, sems.at[len(copies)])
        copies[key].start()

    def wait(*keys):
        for key in keys:
            copies[key].wait()

    def x_cols(key, lo, hi):
        start(key, x_hbm.at[:, pl.ds(lo, hi - lo)], x_v.at[:, pl.ds(lo, hi - lo)])

    def w_cols(key, lo, hi):
        for n, w in enumerate((wq_hbm, wk_hbm, wv_hbm)):
            start((key, n), w.at[:, pl.ds(lo, hi - lo)], w_v.at[n, :, pl.ds(lo, hi - lo)])

    w_cols("wa", 0, T)
    for i in range(NT):
        x_cols(("x", i), i * T, (i + 1) * T)
    start("beta", beta_hbm, beta_ref)
    start("wr", wr_hbm, wr_ref)
    w_cols("wb", T, 3 * T)

    def second_batch():
        w_cols("wc", 3 * T, D)
        x_cols("xc", L, S)
        start("g", wg_hbm, wg_v)

    def third_batch():
        start("wo", wo_hbm, w_v.at[3])
        start("u", wu_hbm, wu_v)
        start("d", wd_hbm, wd_v)

    st = {}

    def layernorm(t):
        x = x_v[:, t * T:(t + 1) * T].astype(F32)
        chains = 4 if t < NT else 1
        m = _colsum(x, chains) / D
        d = x - m
        v = _rb(_colsum(d * d, chains) / D)
        sd = _rb(jnp.sqrt(_rb(v + _rb(jnp.full((1, T), 1e-5, F32)))))
        xn = (_rb(x - _rb(m)) * (1.0 / sd)).astype(BF16)
        xn_s[t] = xn

    def router(t):
        if "wr" not in st:
            st["wr"] = jnp.broadcast_to(wr_ref[...].astype(F32).reshape(1, D), (T, D)).T
        st["r", t] = _rb(_colsum(xn_s[t].astype(F32) * st["wr"]))

    def transpose_w(n, c):
        lo, hi = c * T, min((c + 1) * T, D)
        wt = w_v[n, :, lo:hi].astype(F32).T
        if n == 3:
            wot_s[lo:hi] = wt
            return
        for g in range(lo // GR, (hi - 1) // GR + 1):
            a, b = max(lo, g * GR), min(hi, (g + 1) * GR)
            wt_s[g, n * GR + a - g * GR:n * GR + b - g * GR] = wt[a - lo:b - lo]

    def seg_xn(s):
        return jnp.concatenate([xn_s[s * NT + i] for i in range(NT)], axis=1)

    def project(s, g):
        r = _dot(wt_s[g], seg_xn(s))
        q, k, v = r[0:GR], r[GR:2 * GR], r[2 * GR:3 * GR]
        return dict(q=q, k=k, v=v, kn=_pad_bf16(k).T)

    def mem_mask():
        r, c = _iota((GP, GP), 0), _iota((GP, GP), 1)
        keep = None
        for j in range(HG):
            rows = ((r >= DH * j) & (r < DH * (j + 1))) | (r == GR + j)
            blk = rows & (c >= DH * j) & (c < DH * (j + 1))
            keep = blk if keep is None else keep | blk
        return keep

    def mem_delta(u):
        pk = _pad_bf16(_phi(u["k"]))
        lhs = jnp.concatenate([u["v"], jnp.ones((GP - GR, L), F32)], axis=0)
        acc = None
        for i in range(NT):
            part = _dot_nt(lhs[:, i * T:(i + 1) * T], pk[:, i * T:(i + 1) * T])
            acc = part if acc is None else acc + part
        return jnp.where(mem_mask(), acc, 0.0)

    def mem_read(u, mem, gate):
        r = _dot(mem, _pad_bf16(_phi(u["q"])))
        coef = gate / (r[GR:GP] + 1e-6)
        out = []
        for i in range(NT):
            ci = coef[:, i * T:(i + 1) * T]
            wins = [jnp.broadcast_to(ci[j:j + 1], (24, T)) for j in range(HG)]
            out.append(r[0:GR, i * T:(i + 1) * T] * _merge_heads(wins))
        return out

    def gate_rows(g):
        return g_s[g]

    def finish(accs, gate, mem_i, turn):
        dens = [accs[j][LROW[j]:LROW[j] + 1] for j in range(HG)]
        o = _merge_heads([_rotate(accs[j] * ((1.0 - gate[j:j + 1]) / dens[j]), -j * turn)
                          for j in range(HG)])
        return (o if mem_i is None else o + mem_i), dens

    def out_rows(s, c, idx):
        rows = pl.ds(c * OC, OC)
        cols = pl.ds(s * L if isinstance(s, int) else pl.multiple_of(s * L, L), L)
        a = _dot(wot_s[rows], ot_s[s].astype(BF16))
        tok = _iota((1, L), 1) + s * L
        y0, y1 = (jnp.concatenate([y_s[n, rows]] * NT, axis=1) for n in range(2))
        upd = jnp.where(tok == idx[0], y0, jnp.where(tok == idx[1], y1, 0.0))
        xn = jnp.concatenate([xn_s[s * NT + i, rows] for i in range(NT)], axis=1)
        res = (x_v[rows, cols].astype(F32) + a) + (xn.astype(F32) + upd)
        o_v[rows, cols] = res.astype(BF16)
        return res

    def gates():
        sg = jax.nn.sigmoid(beta_ref[...].astype(F32).reshape(1, H))
        for g in range(NG):
            pick = _iota((8, H), 1) == _iota((8, H), 0) + HG * g
            col = jnp.sum(jnp.where(pick, sg, 0.0), axis=1, keepdims=True)
            g_s[g] = jnp.broadcast_to(col, (8, T))

    def pick(n):
        if n == 0:
            st["r"] = jnp.concatenate([st["r", t] for t in range(S // T)], axis=1)
            st["idx"], st["val"] = [], []
        tok = _iota((1, S), 1)
        best = jnp.max(st["r"], axis=1, keepdims=True)
        i = jnp.clip(jnp.min(jnp.where(st["r"] == best, tok, S)), 0, S - 1)
        st["r"] = jnp.where(tok == i, -jnp.inf, st["r"])
        st["idx"].append(i)
        st["val"].append(best)

    def gather(n):
        i = st["idx"][n]
        hot = ((_iota((8, T), 1) == i % T) & (_iota((8, T), 0) == n)).astype(F32)
        row = _dot_nt(hot, xn_s[i // T])
        st["xs"] = row if n == 0 else st["xs"] + row

    def ffn_in(name, w_ref, c, kt):
        lo, hi = kt * T, min((kt + 1) * T, D)
        part = _dot(st["xs"][:, lo:hi], w_ref[lo:hi, c * FC:(c + 1) * FC])
        st[name] = part if kt == 0 else st[name] + part

    def ffn_act(c):
        g = st["g"]
        h = _rb(g * jax.nn.sigmoid(g) * st["u"])
        for n in range(2):
            for f in range(FC // T):
                h_s[n, c * (FC // T) + f] = jnp.broadcast_to(h[n:n + 1, f * T:(f + 1) * T], (8, T))

    def ffn_out(r):
        acc = [0.0, 0.0]
        for f in range(FF // T):
            w = wd_v[r * 16:(r + 1) * 16, f * T:(f + 1) * T].astype(F32)
            for n in range(2):
                acc[n] = acc[n] + w * jnp.concatenate([h_s[n, f]] * 2, axis=0)
        for n in range(2):
            y = jnp.sum(acc[n], axis=1, keepdims=True) * jax.nn.sigmoid(st["val"][n])
            y_s[n, r * 16:(r + 1) * 16] = jnp.broadcast_to(y, (16, T))
        st["y", r] = (acc[0][0:8] + acc[0][8:16]) + (acc[1][0:8] + acc[1][8:16])

    units, mems = {}, {}
    tiles = [(u, i, c) for u in range(NSEG * NG) for i in CFG["order"] for c in range(i + 1)]
    per_unit = NT * (NT + 1) // 2
    tri = _iota((QB, T), 0) <= _iota((QB, T), 1) % QB
    quarter = _iota((QB, T), 1) // QB
    odd, high = quarter % 2 == 1, quarter >= 2
    slot, head_of_row = _iota((GP, T), 1) // QB, _iota((GP, T), 0) // DH
    rng = dict(lo=jnp.ones((1, T), F32), hi=jnp.ones((1, T), F32), o=jnp.zeros((8, T), F32))

    def do_project(u):
        units[u] = project(u // NG, u % NG)

    def do_mem_read(u):
        gate = jnp.concatenate([gate_rows(u % NG)] * NT, axis=1)
        units[u]["mem"] = mem_read(units[u], mems[u % NG], gate)

    def do_mem_update(u):
        delta = mem_delta(units[u])
        mems[u % NG] = delta if u < NG else mems[u % NG] + delta

    def scores(t):
        u, i, c = tiles[t]
        un = units[u]
        if c == 0:
            q = un["q"][:, i * T:(i + 1) * T] * QSCALE
            qr = _merge_heads([_rotate(q[V0[j]:V0[j] + 24], j) for j in range(HG)])
            un["qr"] = jnp.concatenate([qr, jnp.zeros((GP - GR, T), F32)], axis=0)
            un["qm"] = jnp.concatenate([_head_query(qr, j) for j in range(HG)], axis=1)
        k = un["kn"][c * T:(c + 1) * T]
        if c < i:
            extra = QB if CFG["merge"] and c == i - 1 else 0
            p = jnp.exp2(_dot(un["kn"][c * T:(c + 1) * T + extra], un["qm"]))
            st["p", t] = [p[0:T, j * T:(j + 1) * T].astype(BF16) for j in range(HG)]
            if extra:
                st["p0"] = p[T:]
            return
        p0 = st.pop("p0") if "p0" in st else jnp.exp2(_dot(k[0:QB], un["qm"]))
        e = {}
        for b in (3, 2, 1):
            w = jnp.where(slot == (head_of_row + b) % 4, un["qr"], 0.0).astype(BF16)
            r = jnp.exp2(_dot(k[QB:(b + 1) * QB], w))
            for a in range(1, b + 1):
                blk = r[(a - 1) * QB:a * QB]
                e[a, b] = jnp.where(tri, blk, 0.0) if a == b else blk
        x13 = [jnp.where(high, e[1, 3], e[1, 1]), jnp.where(high, e[1, 1], e[1, 3])]
        x23 = [jnp.where(odd, e[2, 3], e[2, 2]), jnp.where(odd, e[2, 2], e[2, 3])]
        ps = []
        for j in range(HG):
            block = (quarter - j) % 4
            outer = x13[(j + 1) % 4 // 2]
            x1 = jnp.where(odd, e[1, 2], outer) if j % 2 else jnp.where(odd, outer, e[1, 2])
            ps.append(jnp.concatenate(
                [jnp.where(tri | (block > 0), p0[:, j * T:(j + 1) * T], 0.0),
                 jnp.where(block >= 1, x1, 0.0),
                 jnp.where(block >= 2, x23[j % 2], 0.0),
                 jnp.where(block >= 3, e[3, 3], 0.0)], axis=0).astype(BF16))
        st["p", t] = ps

    def values(t):
        u, i, c = tiles[t]
        un = units[u]
        ps = st.pop(("p", t))
        v = un["v"][:, c * T:(c + 1) * T]
        one = 1.0
        for a in st.pop("due", []):
            one = jnp.maximum(jnp.minimum(a, one), one)
        for j in range(HG):
            part = _dot(_head_values(v, j, one), ps[j])
            st["o", j] = part if c == 0 else st["o", j] + part
        if c == i:
            mem_i = un["mem"][i] if "mem" in un else None
            o, dens = finish([st["o", j] for j in range(HG)], gate_rows(u % NG), mem_i, 1)
            ot_s[u // NG, (u % NG) * GR:(u % NG + 1) * GR, i * T:(i + 1) * T] = o
            for l in dens:
                rng["lo"], rng["hi"] = jnp.minimum(rng["lo"], l), jnp.maximum(rng["hi"], l)

    def due(*keys):
        st.setdefault("due", []).append(st[keys])

    def do_out(s, c):
        peak = jnp.max(jnp.abs(out_rows(s, c, st["idx"])).reshape(OC // 8, 8, L), axis=0)
        for i in range(NT):
            rng["o"] = jnp.maximum(rng["o"], peak[:, i * T:(i + 1) * T])
        st["peak", s, c] = rng["o"]
        rows, cols = pl.ds(c * OC, OC), pl.ds(s * L, L)
        start(("o", s, c), o_v.at[rows, cols], o_hbm.at[rows, cols])

    fill = {}

    def at(step, fn, *args):
        fill.setdefault(step, []).append((fn, args))

    nu = NSEG * NG
    for u in range(nu):
        t0 = u * per_unit
        if u + 1 < nu:
            at(t0 + (CFG["proj"] if u else 5), do_project, u + 1)
        if u >= NG:
            at(t0 + CFG["read"], do_mem_read, u)
        if u < nu - NG:
            at(t0 + CFG["upd"], do_mem_update, u)
    at(CFG["s1"], second_batch)
    at(CFG["s1"], wait, ("wb", 0), ("wb", 1), ("wb", 2), "beta", "wr")
    at(CFG["s1"], gates)
    step = 4 * per_unit + CFG["s2"]
    at(step, wait, "xc", ("wc", 0), ("wc", 1))
    at(step, third_batch)
    at(step, wait, ("wc", 2))
    for c in range(1, 5):
        for n in range(3):
            at(max((T * c // GR - 1) * per_unit + 2, CFG["s1"]), transpose_w, n, c)
    for t in range(S // T):
        if t < NT:
            at(per_unit + CFG["r0"] + t * 5, router, t)
            at(per_unit + CFG["r0"] + t * 5, due, "r", t)
        else:
            at(step, layernorm, t)
            at(step, router, t)
            at(4 * per_unit + 2 + CFG["l0"] + (t - NT) * CFG["ls"], due, "r", t)
    for n in range(2):
        at((11 + n) * per_unit + 6, pick, n)
        at((13 + n) * per_unit + CFG["gstep"], gather, n)
    step = CFG["ffn0"] * per_unit + CFG["wstep"]
    at(step, wait, "wo", "g", "u", "d")
    for c in range(5):
        at(step + c * per_unit, transpose_w, 3, c)
    for c in range(FF // FC):
        for name, w in (("g", wg_v), ("u", wu_v)):
            for kt in range(5):
                at(step, ffn_in, name, w, c, kt)
                step += 1
        at(step - 1, ffn_act, c)
    step += 2
    for r in range(D // 16):
        at(step + int(r * CFG["ys"]), ffn_out, r)
        at(step + int(r * CFG["ys"]), due, "y", r)
    step += int(D // 16 * CFG["ys"])
    chunks = [(s, c) for s in range(NSEG - 1) for c in range(D // OC)]
    gap = (len(tiles) - step - 6) // (len(chunks) - 1)
    for n, (s, c) in enumerate(chunks[:-1]):
        at(step + 6 + n * gap, do_out, s, c)
        if CFG["odue"]:
            at(step + 6 + n * gap + CFG["odue"], due, "peak", s, c)

    wait(("wa", 0), ("wa", 1), ("wa", 2))
    for n in range(3):
        transpose_w(n, 0)
    for batch in ((0, 1), (2,), (3,)):
        wait(*[("x", i) for i in batch])
        for i in batch:
            layernorm(i)
    do_project(0)
    lag = CFG["lag"]
    for t in range(len(tiles) + lag):
        for fn, args in fill.pop(t, []):
            fn(*args)
        if t < len(tiles):
            scores(t)
        if t == len(tiles):
            do_out(*chunks[-1])
        if t >= lag:
            values(t - lag)
    assert not fill
    for c in range(D // OC):
        do_out(NSEG - 1, c)
    safe = (jnp.min(rng["lo"]) >= L_LO) & (jnp.max(rng["hi"]) <= L_HI) & (jnp.max(rng["o"]) <= O_HI)
    wait(*[key for key in copies if key[0] == "o" and key != "o"])

    @pl.when(jnp.logical_not(safe))
    def _():
        m_s[...] = jnp.zeros(m_s.shape, F32)

        def unit(u, carry):
            s, g = u // NG, u % NG
            un = project(s, g)
            gate = gate_rows(g)
            mem = mem_read(un, m_s[g], jnp.concatenate([gate] * NT, axis=1))
            for i in range(NT):
                nk = (i + 1) * T
                q = un["q"][:, i * T:nk] * QSCALE
                keep = _iota((nk, T), 0) <= _iota((nk, T), 1) + i * T
                accs = []
                for j in range(HG):
                    sc = jnp.where(keep, _dot(un["kn"][0:nk], _head_query(q, j)), -jnp.inf)
                    p = jnp.exp2(sc - jnp.max(sc, axis=0, keepdims=True))
                    accs.append(_dot(_head_values(un["v"][:, 0:nk], j), p.astype(BF16)))
                o, _ = finish(accs, gate, mem[i], 0)
                ot_s[s, pl.ds(pl.multiple_of(g * GR, 8), GR), i * T:nk] = o
            m_s[g] += mem_delta(un)
            return carry

        lax.fori_loop(0, nu, unit, 0)

        def segment(s, carry):
            for c in range(D // OC):
                out_rows(s, c, st["idx"])
            return carry

        lax.fori_loop(0, NSEG, segment, 0)
        redo = pltpu.make_async_copy(o_v, o_hbm, sems.at[0])
        redo.start()
        redo.wait()


@jax.jit
def pallas_parallel_sum__memory_aug_infini_attn__moe_arch_mod__prompt_kernel(
    A_x: jax.Array,
    A_wq: jax.Array,
    A_wk: jax.Array,
    A_wv: jax.Array,
    A_wo: jax.Array,
    A_beta: jax.Array,
    B_x: jax.Array,
    B_w_r: jax.Array,
    B_w_gate: jax.Array,
    B_w_up: jax.Array,
    B_w_down: jax.Array,
):
    del B_x
    hbm = pl.BlockSpec(memory_space=pltpu.HBM)
    nsem = 20 + NSEG * (D // OC)
    out = pl.pallas_call(
        _kernel,
        out_shape=jax.ShapeDtypeStruct((D, S), BF16),
        in_specs=[hbm] * 10,
        out_specs=hbm,
        scratch_shapes=[
            pltpu.VMEM((H,), BF16),
            pltpu.VMEM((D,), BF16),
            pltpu.VMEM((D, S), BF16),
            pltpu.VMEM((4, D, D), BF16),
            pltpu.VMEM((D, FF), BF16),
            pltpu.VMEM((D, FF), BF16),
            pltpu.VMEM((D, FF), BF16),
            pltpu.VMEM((S // T, D, T), BF16),
            pltpu.VMEM((NG, 3 * GR, D), F32),
            pltpu.VMEM((D, D), F32),
            pltpu.VMEM((NSEG, D, L), F32),
            pltpu.VMEM((D, S), BF16),
            pltpu.VMEM((2, FF // T, 8, T), F32),
            pltpu.VMEM((2, D, T), F32),
            pltpu.VMEM((NG, 8, T), F32),
            pltpu.VMEM((NG, GP, GP), F32),
            pltpu.SemaphoreType.DMA((nsem,)),
        ],
        compiler_params=pltpu.CompilerParams(vmem_limit_bytes=100 * 1024 * 1024),
        name="infini_mod",
    )(A_x.reshape(S, D).T, A_wq, A_wk, A_wv, A_wo, A_beta, B_w_r, B_w_gate, B_w_up, B_w_down.T)
    return out.T.reshape(1, S, D)
```

```python
import jax
import jax.numpy as jnp
from jax import lax
import jax.experimental.pallas as pl
import jax.experimental.pallas.tpu as pltpu

F32, BF16 = jnp.float32, jnp.bfloat16
S, D, H, DH, NSEG, L, FF = 2048, 576, 32, 18, 4, 512, 4608
T = 128
QB = T // 4
NT = L // T
HG = 4
GR = HG * DH
GP = 80
NG = H // HG
LOG2E = 1.4426950408889634
QSCALE = DH ** -0.5 * LOG2E
L_LO, L_HI, O_HI = 2.0 ** -40, 2.0 ** 40, 3.0e38
FC = 512
OC = 144
NT_DIMS = (((1,), (1,)), ((), ()))
V0 = (0, 16, 32, 48)
LROW = (23, 23, 23, 0)
CFG = dict(order=(2, 0, 3, 1), lag=2, proj=3, read=0, upd=9, merge=1, ffn0=16, wstep=7, odue=2, gstep=6, r0=4, l0=5, ls=5, ys=1.0, p1=5, s1=2, s2=-3)


def _iota(shape, dim):
    return lax.broadcasted_iota(jnp.int32, shape, dim)


def _dot(a, b):
    return jnp.dot(a, b, preferred_element_type=F32)


def _dot_nt(a, b):
    return lax.dot_general(a, b, NT_DIMS, preferred_element_type=F32)


def _rb(x):
    return x.astype(BF16).astype(F32)


def _colsum(x, chains=1):
    n = x.shape[0] // chains
    p = [jnp.sum(x[i * n:(i + 1) * n].reshape(n // 8, 8, x.shape[1]), axis=0) for i in range(chains)]
    return jnp.sum(sum(p[1:], p[0]), axis=0, keepdims=True)


def _phi(t):
    return jnp.where(t > 0, t + 1.0, jnp.exp(t))


def _pad_bf16(a):
    return jnp.concatenate([a, jnp.zeros((GP - GR, a.shape[1]), F32)], axis=0).astype(BF16)


def _merge_heads(wins):
    a, b, c, e = wins
    r = _iota((8, T), 0)
    return jnp.concatenate(
        [a[0:16], jnp.where(r < 2, a[16:24], b[0:8]), b[8:16],
         jnp.where(r < 4, b[16:24], c[0:8]), c[8:16],
         jnp.where(r < 6, c[16:24], e[0:8]), e[8:24]], axis=0)


def _rotate(a, quarters):
    return pltpu.roll(a, quarters % 4 * QB, 1) if quarters % 4 else a


def _head_query(q, j):
    lo, hi = DH * j, DH * (j + 1)
    a, b = lo // 16 * 16, min(lo // 16 * 16 + 32, GR)
    r = _iota((b - a, T), 0) + a
    parts = [jnp.where((r >= lo) & (r < hi), q[a:b], 0.0)]
    if a:
        parts = [jnp.zeros((a, T), F32)] + parts
    if b < GP:
        parts = parts + [jnp.zeros((GP - b, T), F32)]
    return jnp.concatenate(parts, axis=0).astype(BF16)


def _head_values(v, j, one=1.0):
    w = v[V0[j]:V0[j] + 24]
    r = _iota((8, v.shape[1]), 0)
    if LROW[j] == 0:
        return jnp.concatenate([jnp.where(r == 0, one, w[0:8]), w[8:24]], axis=0)
    return jnp.concatenate([w[0:16], jnp.where(r == 7, one, w[16:24])], axis=0)


def _kernel(x_hbm, wq_hbm, wk_hbm, wv_hbm, wo_hbm, beta_hbm, wr_hbm, wg_hbm, wu_hbm, wd_hbm,
            o_hbm, beta_ref, wr_ref, x_v, w_v, wg_v, wu_v, wd_v, xn_s, wt_s, wot_s, ot_s, o_v, h_s, y_s, g_s, m_s, sems):
    copies = {}

    def start(key, src, dst):
        copies[key] = pltpu.make_async_copy(src, dst, sems.at[len(copies)])
        copies[key].start()

    def wait(*keys):
        for key in keys:
            copies[key].wait()

    def x_cols(key, lo, hi):
        start(key, x_hbm.at[:, pl.ds(lo, hi - lo)], x_v.at[:, pl.ds(lo, hi - lo)])

    def w_cols(key, lo, hi):
        for n, w in ((1, wk_hbm), (0, wq_hbm), (2, wv_hbm)):
            start((key, n), w.at[:, pl.ds(lo, hi - lo)], w_v.at[n, :, pl.ds(lo, hi - lo)])

    for i in range(NT):
        x_cols(("x", i), i * T, (i + 1) * T)
    w_cols("wa", 0, T)
    start("beta", beta_hbm, beta_ref)
    start("wr", wr_hbm, wr_ref)

    def second_batch():
        w_cols("wc", 2 * T, D)
        x_cols("xc", L, S)
        start("g", wg_hbm, wg_v)

    def third_batch():
        start("wo", wo_hbm, w_v.at[3])
        start("u", wu_hbm, wu_v)
        start("d", wd_hbm, wd_v)

    st = {}

    def layernorm(t):
        x = x_v[:, t * T:(t + 1) * T].astype(F32)
        chains = 4 if t < NT else 1
        m = _colsum(x, chains) / D
        d = x - m
        v = _rb(_colsum(d * d, chains) / D)
        sd = _rb(jnp.sqrt(_rb(v + _rb(jnp.full((1, T), 1e-5, F32)))))
        xn = (_rb(x - _rb(m)) * (1.0 / sd)).astype(BF16)
        xn_s[t] = xn

    def router(t):
        if "wr" not in st:
            st["wr"] = jnp.broadcast_to(wr_ref[...].astype(F32).reshape(1, D), (T, D)).T
        st["r", t] = _rb(_colsum(xn_s[t].astype(F32) * st["wr"]))

    def transpose_w(n, c):
        lo, hi = c * T, min((c + 1) * T, D)
        wt = w_v[n, :, lo:hi].astype(F32).T
        if n == 3:
            wot_s[lo:hi] = wt
            return
        for g in range(lo // GR, (hi - 1) // GR + 1):
            a, b = max(lo, g * GR), min(hi, (g + 1) * GR)
            wt_s[g, n * GR + a - g * GR:n * GR + b - g * GR] = wt[a - lo:b - lo]

    def seg_xn(s):
        return jnp.concatenate([xn_s[s * NT + i] for i in range(NT)], axis=1)

    def unit_of(q, k, v):
        return dict(q=q, k=k, v=v, kn=_pad_bf16(k).T)

    def project(s, g):
        r = _dot(wt_s[g], seg_xn(s))
        return unit_of(r[0:GR], r[GR:2 * GR], r[2 * GR:3 * GR])

    def mem_mask():
        r, c = _iota((GP, GP), 0), _iota((GP, GP), 1)
        keep = None
        for j in range(HG):
            rows = ((r >= DH * j) & (r < DH * (j + 1))) | (r == GR + j)
            blk = rows & (c >= DH * j) & (c < DH * (j + 1))
            keep = blk if keep is None else keep | blk
        return keep

    def mem_delta(u):
        pk = _pad_bf16(_phi(u["k"]))
        lhs = jnp.concatenate([u["v"], jnp.ones((GP - GR, L), F32)], axis=0)
        acc = None
        for i in range(NT):
            part = _dot_nt(lhs[:, i * T:(i + 1) * T], pk[:, i * T:(i + 1) * T])
            acc = part if acc is None else acc + part
        return jnp.where(mem_mask(), acc, 0.0)

    def mem_read(u, mem, gate):
        r = _dot(mem, _pad_bf16(_phi(u["q"])))
        coef = gate / (r[GR:GP] + 1e-6)
        out = []
        for i in range(NT):
            ci = coef[:, i * T:(i + 1) * T]
            wins = [jnp.broadcast_to(ci[j:j + 1], (24, T)) for j in range(HG)]
            out.append(r[0:GR, i * T:(i + 1) * T] * _merge_heads(wins))
        return out

    def gate_rows(g):
        return g_s[g]

    def finish(accs, gate, mem_i, turn):
        dens = [accs[j][LROW[j]:LROW[j] + 1] for j in range(HG)]
        o = _merge_heads([_rotate(accs[j] * ((1.0 - gate[j:j + 1]) / dens[j]), -j * turn)
                          for j in range(HG)])
        return (o if mem_i is None else o + mem_i), dens

    def out_rows(s, c, idx):
        rows = pl.ds(c * OC, OC)
        cols = pl.ds(s * L if isinstance(s, int) else pl.multiple_of(s * L, L), L)
        a = _dot(wot_s[rows], ot_s[s].astype(BF16))
        tok = _iota((1, L), 1) + s * L
        y0, y1 = (jnp.concatenate([y_s[n, rows]] * NT, axis=1) for n in range(2))
        upd = jnp.where(tok == idx[0], y0, jnp.where(tok == idx[1], y1, 0.0))
        xn = jnp.concatenate([xn_s[s * NT + i, rows] for i in range(NT)], axis=1)
        res = (x_v[rows, cols].astype(F32) + a) + (xn.astype(F32) + upd)
        o_v[rows, cols] = res.astype(BF16)
        return res

    def gates():
        sg = jax.nn.sigmoid(beta_ref[...].astype(F32).reshape(1, H))
        for g in range(NG):
            pick = _iota((8, H), 1) == _iota((8, H), 0) + HG * g
            col = jnp.sum(jnp.where(pick, sg, 0.0), axis=1, keepdims=True)
            g_s[g] = jnp.broadcast_to(col, (8, T))

    def pick(n):
        if n == 0:
            st["r"] = jnp.concatenate([st["r", t] for t in range(S // T)], axis=1)
            st["idx"], st["val"] = [], []
        tok = _iota((1, S), 1)
        best = jnp.max(st["r"], axis=1, keepdims=True)
        i = jnp.clip(jnp.min(jnp.where(st["r"] == best, tok, S)), 0, S - 1)
        st["r"] = jnp.where(tok == i, -jnp.inf, st["r"])
        st["idx"].append(i)
        st["val"].append(best)

    def gather(n):
        i = st["idx"][n]
        hot = ((_iota((8, T), 1) == i % T) & (_iota((8, T), 0) == n)).astype(F32)
        row = _dot_nt(hot, xn_s[i // T])
        st["xs"] = row if n == 0 else st["xs"] + row

    def ffn_in(name, w_ref, c, kt):
        lo, hi = kt * T, min((kt + 1) * T, D)
        part = _dot(st["xs"][:, lo:hi], w_ref[lo:hi, c * FC:(c + 1) * FC])
        st[name] = part if kt == 0 else st[name] + part

    def ffn_act(c):
        g = st["g"]
        h = _rb(g * jax.nn.sigmoid(g) * st["u"])
        for n in range(2):
            for f in range(FC // T):
                h_s[n, c * (FC // T) + f] = jnp.broadcast_to(h[n:n + 1, f * T:(f + 1) * T], (8, T))

    def ffn_out(r):
        acc = [0.0, 0.0]
        for f in range(FF // T):
            w = wd_v[r * 16:(r + 1) * 16, f * T:(f + 1) * T].astype(F32)
            for n in range(2):
                acc[n] = acc[n] + w * jnp.concatenate([h_s[n, f]] * 2, axis=0)
        for n in range(2):
            y = jnp.sum(acc[n], axis=1, keepdims=True) * jax.nn.sigmoid(st["val"][n])
            y_s[n, r * 16:(r + 1) * 16] = jnp.broadcast_to(y, (16, T))
        st["y", r] = (acc[0][0:8] + acc[0][8:16]) + (acc[1][0:8] + acc[1][8:16])

    units, mems = {}, {}
    tiles = [(u, i, c) for u in range(NSEG * NG) for i in CFG["order"] for c in range(i + 1)]
    per_unit = NT * (NT + 1) // 2
    tri = _iota((QB, T), 0) <= _iota((QB, T), 1) % QB
    quarter = _iota((QB, T), 1) // QB
    odd, high = quarter % 2 == 1, quarter >= 2
    slot, head_of_row = _iota((GP, T), 1) // QB, _iota((GP, T), 0) // DH
    rng = dict(lo=jnp.ones((1, T), F32), hi=jnp.ones((1, T), F32), o=jnp.zeros((8, T), F32))

    def do_project(u):
        units[u] = project(u // NG, u % NG)

    def do_mem_read(u):
        gate = jnp.concatenate([gate_rows(u % NG)] * NT, axis=1)
        units[u]["mem"] = mem_read(units[u], mems[u % NG], gate)

    def do_mem_update(u):
        delta = mem_delta(units[u])
        mems[u % NG] = delta if u < NG else mems[u % NG] + delta

    def scores(t):
        u, i, c = tiles[t]
        un = units[u]
        if c == 0:
            q = un["q"][:, i * T:(i + 1) * T] * QSCALE
            qr = _merge_heads([_rotate(q[V0[j]:V0[j] + 24], j) for j in range(HG)])
            un["qr"] = jnp.concatenate([qr, jnp.zeros((GP - GR, T), F32)], axis=0)
            un["qm"] = jnp.concatenate([_head_query(qr, j) for j in range(HG)], axis=1)
        k = un["kn"][c * T:(c + 1) * T]
        if c < i:
            extra = QB if CFG["merge"] and c == i - 1 else 0
            p = jnp.exp2(_dot(un["kn"][c * T:(c + 1) * T + extra], un["qm"]))
            st["p", t] = [p[0:T, j * T:(j + 1) * T].astype(BF16) for j in range(HG)]
            if extra:
                st["p0"] = p[T:]
            return
        p0 = st.pop("p0") if "p0" in st else jnp.exp2(_dot(k[0:QB], un["qm"]))
        e = {}
        for b in (3, 2, 1):
            w = jnp.where(slot == (head_of_row + b) % 4, un["qr"], 0.0).astype(BF16)
            r = jnp.exp2(_dot(k[QB:(b + 1) * QB], w))
            for a in range(1, b + 1):
                blk = r[(a - 1) * QB:a * QB]
                e[a, b] = jnp.where(tri, blk, 0.0) if a == b else blk
        x13 = [jnp.where(high, e[1, 3], e[1, 1]), jnp.where(high, e[1, 1], e[1, 3])]
        x23 = [jnp.where(odd, e[2, 3], e[2, 2]), jnp.where(odd, e[2, 2], e[2, 3])]
        ps = []
        for j in range(HG):
            block = (quarter - j) % 4
            outer = x13[(j + 1) % 4 // 2]
            x1 = jnp.where(odd, e[1, 2], outer) if j % 2 else jnp.where(odd, outer, e[1, 2])
            ps.append(jnp.concatenate(
                [jnp.where(tri | (block > 0), p0[:, j * T:(j + 1) * T], 0.0),
                 jnp.where(block >= 1, x1, 0.0),
                 jnp.where(block >= 2, x23[j % 2], 0.0),
                 jnp.where(block >= 3, e[3, 3], 0.0)], axis=0).astype(BF16))
        st["p", t] = ps

    def values(t):
        u, i, c = tiles[t]
        un = units[u]
        ps = st.pop(("p", t))
        v = un["v"][:, c * T:(c + 1) * T]
        one = 1.0
        for a in st.pop("due", []):
            one = jnp.maximum(jnp.minimum(a, one), one)
        for j in range(HG):
            part = _dot(_head_values(v, j, one), ps[j])
            st["o", j] = part if c == 0 else st["o", j] + part
        if c == i:
            mem_i = un["mem"][i] if "mem" in un else None
            o, dens = finish([st["o", j] for j in range(HG)], gate_rows(u % NG), mem_i, 1)
            ot_s[u // NG, (u % NG) * GR:(u % NG + 1) * GR, i * T:(i + 1) * T] = o
            for l in dens:
                rng["lo"], rng["hi"] = jnp.minimum(rng["lo"], l), jnp.maximum(rng["hi"], l)

    def due(*keys):
        st.setdefault("due", []).append(st[keys])

    def do_out(s, c):
        peak = jnp.max(jnp.abs(out_rows(s, c, st["idx"])).reshape(OC // 8, 8, L), axis=0)
        for i in range(NT):
            rng["o"] = jnp.maximum(rng["o"], peak[:, i * T:(i + 1) * T])
        st["peak", s, c] = rng["o"]
        rows, cols = pl.ds(c * OC, OC), pl.ds(s * L, L)
        start(("o", s, c), o_v.at[rows, cols], o_hbm.at[rows, cols])

    fill = {}

    def at(step, fn, *args):
        fill.setdefault(step, []).append((fn, args))

    nu = NSEG * NG
    for u in range(nu):
        t0 = u * per_unit
        if u + 1 < nu:
            at(t0 + (CFG["proj"] if u else CFG["p1"]), do_project, u + 1)
        if u >= NG:
            at(t0 + CFG["read"], do_mem_read, u)
        if u < nu - NG:
            at(t0 + CFG["upd"], do_mem_update, u)
    at(CFG["s1"], second_batch)
    at(CFG["s1"], wait, ("wb", 0), ("wb", 1), ("wb", 2), "beta", "wr")
    at(CFG["s1"], gates)
    step = 4 * per_unit + CFG["s2"]
    at(2 * per_unit + 1, wait, ("wc", 0), ("wc", 1), ("wc", 2))
    at(step, third_batch)
    at(step, wait, "xc")
    for c in range(1, 5):
        for n in range(3):
            at(max((T * c // GR - 1) * per_unit + 2, CFG["s1"]), transpose_w, n, c)
    for t in range(S // T):
        if t < NT:
            at(per_unit + CFG["r0"] + t * 5, router, t)
            at(per_unit + CFG["r0"] + t * 5, due, "r", t)
        else:
            at(step, layernorm, t)
            at(step, router, t)
            at(4 * per_unit + 2 + CFG["l0"] + (t - NT) * CFG["ls"], due, "r", t)
    for n in range(2):
        at((11 + n) * per_unit + 6, pick, n)
        at((13 + n) * per_unit + CFG["gstep"], gather, n)
    step = CFG["ffn0"] * per_unit + CFG["wstep"]
    at(step, wait, "wo", "g", "u", "d")
    for c in range(5):
        at(step + c * per_unit, transpose_w, 3, c)
    for c in range(FF // FC):
        for name, w in (("g", wg_v), ("u", wu_v)):
            for kt in range(5):
                at(step, ffn_in, name, w, c, kt)
                step += 1
        at(step - 1, ffn_act, c)
    step += 2
    for r in range(D // 16):
        at(step + int(r * CFG["ys"]), ffn_out, r)
        at(step + int(r * CFG["ys"]), due, "y", r)
    step += int(D // 16 * CFG["ys"])
    chunks = [(s, c) for s in range(NSEG - 1) for c in range(D // OC)]
    gap = (len(tiles) - step - 6) // (len(chunks) - 1)
    for n, (s, c) in enumerate(chunks[:-1]):
        at(step + 6 + n * gap, do_out, s, c)
        if CFG["odue"]:
            at(step + 6 + n * gap + CFG["odue"], due, "peak", s, c)

    for i in range(NT - 1):
        wait(("x", i))
        layernorm(i)
    wait(("x", NT - 1))
    w_cols("wb", T, 2 * T)
    wait(("wa", 1))
    layernorm(NT - 1)
    transpose_w(1, 0)
    wait(("wa", 0))
    transpose_w(0, 0)
    k0 = _dot(wt_s[0, GR:2 * GR], seg_xn(0))
    wait(("wa", 2))
    transpose_w(2, 0)
    units[0] = unit_of(_dot(wt_s[0, 0:GR], seg_xn(0)), k0, _dot(wt_s[0, 2 * GR:3 * GR], seg_xn(0)))
    lag = CFG["lag"]
    for t in range(len(tiles) + lag):
        for fn, args in fill.pop(t, []):
            fn(*args)
        if t < len(tiles):
            scores(t)
        if t == len(tiles):
            do_out(*chunks[-1])
        if t >= lag:
            values(t - lag)
    assert not fill
    for c in range(D // OC):
        do_out(NSEG - 1, c)
    written = [key for key in copies if key[0] == "o"]
    wait(*written[:-1])
    safe = (jnp.min(rng["lo"]) >= L_LO) & (jnp.max(rng["hi"]) <= L_HI) & (jnp.max(rng["o"]) <= O_HI)
    wait(written[-1])

    @pl.when(jnp.logical_not(safe))
    def _():
        m_s[...] = jnp.zeros(m_s.shape, F32)

        def unit(u, carry):
            s, g = u // NG, u % NG
            un = project(s, g)
            gate = gate_rows(g)
            mem = mem_read(un, m_s[g], jnp.concatenate([gate] * NT, axis=1))
            for i in range(NT):
                nk = (i + 1) * T
                q = un["q"][:, i * T:nk] * QSCALE
                keep = _iota((nk, T), 0) <= _iota((nk, T), 1) + i * T
                accs = []
                for j in range(HG):
                    sc = jnp.where(keep, _dot(un["kn"][0:nk], _head_query(q, j)), -jnp.inf)
                    p = jnp.exp2(sc - jnp.max(sc, axis=0, keepdims=True))
                    accs.append(_dot(_head_values(un["v"][:, 0:nk], j), p.astype(BF16)))
                o, _ = finish(accs, gate, mem[i], 0)
                ot_s[s, pl.ds(pl.multiple_of(g * GR, 8), GR), i * T:nk] = o
            m_s[g] += mem_delta(un)
            return carry

        lax.fori_loop(0, nu, unit, 0)

        def segment(s, carry):
            for c in range(D // OC):
                out_rows(s, c, st["idx"])
            return carry

        lax.fori_loop(0, NSEG, segment, 0)
        redo = pltpu.make_async_copy(o_v, o_hbm, sems.at[0])
        redo.start()
        redo.wait()


@jax.jit
def pallas_parallel_sum__memory_aug_infini_attn__moe_arch_mod__prompt_kernel(
    A_x: jax.Array,
    A_wq: jax.Array,
    A_wk: jax.Array,
    A_wv: jax.Array,
    A_wo: jax.Array,
    A_beta: jax.Array,
    B_x: jax.Array,
    B_w_r: jax.Array,
    B_w_gate: jax.Array,
    B_w_up: jax.Array,
    B_w_down: jax.Array,
):
    del B_x
    hbm = pl.BlockSpec(memory_space=pltpu.HBM)
    nsem = 20 + NSEG * (D // OC)
    out = pl.pallas_call(
        _kernel,
        out_shape=jax.ShapeDtypeStruct((D, S), BF16),
        in_specs=[hbm] * 10,
        out_specs=hbm,
        scratch_shapes=[
            pltpu.VMEM((H,), BF16),
            pltpu.VMEM((D,), BF16),
            pltpu.VMEM((D, S), BF16),
            pltpu.VMEM((4, D, D), BF16),
            pltpu.VMEM((D, FF), BF16),
            pltpu.VMEM((D, FF), BF16),
            pltpu.VMEM((D, FF), BF16),
            pltpu.VMEM((S // T, D, T), BF16),
            pltpu.VMEM((NG, 3 * GR, D), F32),
            pltpu.VMEM((D, D), F32),
            pltpu.VMEM((NSEG, D, L), F32),
            pltpu.VMEM((D, S), BF16),
            pltpu.VMEM((2, FF // T, 8, T), F32),
            pltpu.VMEM((2, D, T), F32),
            pltpu.VMEM((NG, 8, T), F32),
            pltpu.VMEM((NG, GP, GP), F32),
            pltpu.SemaphoreType.DMA((nsem,)),
        ],
        compiler_params=pltpu.CompilerParams(vmem_limit_bytes=100 * 1024 * 1024),
        name="infini_mod",
    )(A_x.reshape(S, D).T, A_wq, A_wk, A_wv, A_wo, A_beta, B_w_r, B_w_gate, B_w_up, B_w_down.T)
    return out.T.reshape(1, S, D)
```

```python
import jax
import jax.numpy as jnp
from jax import lax
import jax.experimental.pallas as pl
import jax.experimental.pallas.tpu as pltpu

F32, BF16 = jnp.float32, jnp.bfloat16
S, D, H, DH, NSEG, L, FF = 2048, 576, 32, 18, 4, 512, 4608
T = 128
QB = T // 4
NT = L // T
HG = 4
GR = HG * DH
GP = 80
NG = H // HG
LOG2E = 1.4426950408889634
QSCALE = DH ** -0.5 * LOG2E
L_LO, L_HI, O_HI = 2.0 ** -40, 2.0 ** 40, 3.0e38
FC = 512
OC = 144
NT_DIMS = (((1,), (1,)), ((), ()))
V0 = (0, 16, 32, 48)
LROW = (23, 23, 23, 0)
ORDER = (2, 0, 3, 1)
STEPS = NT * (NT + 1) // 2
LAG = 2


def _iota(shape, dim):
    return lax.broadcasted_iota(jnp.int32, shape, dim)


def _dot(a, b):
    return jnp.dot(a, b, preferred_element_type=F32)


def _dot_nt(a, b):
    return lax.dot_general(a, b, NT_DIMS, preferred_element_type=F32)


def _rb(x):
    return x.astype(BF16).astype(F32)


def _colsum(x, chains=1):
    n = x.shape[0] // chains
    p = [jnp.sum(x[i * n:(i + 1) * n].reshape(n // 8, 8, x.shape[1]), axis=0) for i in range(chains)]
    return jnp.sum(sum(p[1:], p[0]), axis=0, keepdims=True)


def _phi(t):
    return jnp.where(t > 0, t + 1.0, jnp.exp(t))


def _pad_bf16(a):
    return jnp.concatenate([a, jnp.zeros((GP - GR, a.shape[1]), F32)], axis=0).astype(BF16)


def _merge_heads(wins):
    a, b, c, e = wins
    r = _iota((8, T), 0)
    return jnp.concatenate(
        [a[0:16], jnp.where(r < 2, a[16:24], b[0:8]), b[8:16],
         jnp.where(r < 4, b[16:24], c[0:8]), c[8:16],
         jnp.where(r < 6, c[16:24], e[0:8]), e[8:24]], axis=0)


def _rotate(a, quarters):
    return pltpu.roll(a, quarters % 4 * QB, 1) if quarters % 4 else a


def _head_query(q, j):
    lo, hi = DH * j, DH * (j + 1)
    a, b = lo // 16 * 16, min(lo // 16 * 16 + 32, GR)
    r = _iota((b - a, T), 0) + a
    parts = [jnp.where((r >= lo) & (r < hi), q[a:b], 0.0)]
    if a:
        parts = [jnp.zeros((a, T), F32)] + parts
    if b < GP:
        parts = parts + [jnp.zeros((GP - b, T), F32)]
    return jnp.concatenate(parts, axis=0).astype(BF16)


def _head_values(v, j, one=1.0):
    w = v[V0[j]:V0[j] + 24]
    r = _iota((8, v.shape[1]), 0)
    if LROW[j] == 0:
        return jnp.concatenate([jnp.where(r == 0, one, w[0:8]), w[8:24]], axis=0)
    return jnp.concatenate([w[0:16], jnp.where(r == 7, one, w[16:24])], axis=0)


def _kernel(x_hbm, wq_hbm, wk_hbm, wv_hbm, wo_hbm, beta_hbm, wr_hbm, wg_hbm, wu_hbm, wd_hbm,
            o_hbm, beta_ref, wr_ref, x_v, w_v, wg_v, wu_v, wd_v,
            xn_s, wt_s, wot_s, ot_s, o_v, h_s, y_s, g_s, m_s, sems):
    copies = {}

    def start(key, src, dst):
        copies[key] = pltpu.make_async_copy(src, dst, sems.at[len(copies)])
        copies[key].start()

    def wait(*keys):
        for key in keys:
            copies[key].wait()

    def x_cols(key, lo, hi):
        start(key, x_hbm.at[:, pl.ds(lo, hi - lo)], x_v.at[:, pl.ds(lo, hi - lo)])

    def w_cols(key, lo, hi):
        for n, w in ((1, wk_hbm), (0, wq_hbm), (2, wv_hbm)):
            start((key, n), w.at[:, pl.ds(lo, hi - lo)], w_v.at[n, :, pl.ds(lo, hi - lo)])

    for i in range(NT):
        x_cols(("x", i), i * T, (i + 1) * T)
    w_cols("wa", 0, T)
    start("beta", beta_hbm, beta_ref)
    start("wr", wr_hbm, wr_ref)

    def second_batch():
        w_cols("wc", 2 * T, D)
        x_cols("xc", L, S)
        start("g", wg_hbm, wg_v)

    def third_batch():
        start("wo", wo_hbm, w_v.at[3])
        start("u", wu_hbm, wu_v)
        start("d", wd_hbm, wd_v)

    st = {}

    def layernorm(t):
        x = x_v[:, t * T:(t + 1) * T].astype(F32)
        chains = 4 if t < NT else 1
        m = _colsum(x, chains) / D
        d = x - m
        v = _rb(_colsum(d * d, chains) / D)
        sd = _rb(jnp.sqrt(_rb(v + _rb(jnp.full((1, T), 1e-5, F32)))))
        xn_s[t] = (_rb(x - _rb(m)) * (1.0 / sd)).astype(BF16)

    def router(t):
        if "wr" not in st:
            st["wr"] = jnp.broadcast_to(wr_ref[...].astype(F32).reshape(1, D), (T, D)).T
        st["r", t] = _rb(_colsum(xn_s[t].astype(F32) * st["wr"]))

    def transpose_w(n, c):
        lo, hi = c * T, min((c + 1) * T, D)
        wt = w_v[n, :, lo:hi].astype(F32).T
        if n == 3:
            wot_s[lo:hi] = wt
            return
        for g in range(lo // GR, (hi - 1) // GR + 1):
            a, b = max(lo, g * GR), min(hi, (g + 1) * GR)
            wt_s[g, n * GR + a - g * GR:n * GR + b - g * GR] = wt[a - lo:b - lo]

    def seg_xn(s):
        return jnp.concatenate([xn_s[s * NT + i] for i in range(NT)], axis=1)

    def unit_of(q, k, v):
        return dict(q=q, k=k, v=v, kn=_pad_bf16(k).T)

    def project(s, g):
        r = _dot(wt_s[g], seg_xn(s))
        return unit_of(r[0:GR], r[GR:2 * GR], r[2 * GR:3 * GR])

    def mem_mask():
        r, c = _iota((GP, GP), 0), _iota((GP, GP), 1)
        keep = None
        for j in range(HG):
            rows = ((r >= DH * j) & (r < DH * (j + 1))) | (r == GR + j)
            blk = rows & (c >= DH * j) & (c < DH * (j + 1))
            keep = blk if keep is None else keep | blk
        return keep

    def mem_delta(u):
        pk = _pad_bf16(_phi(u["k"]))
        lhs = jnp.concatenate([u["v"], jnp.ones((GP - GR, L), F32)], axis=0)
        acc = None
        for i in range(NT):
            part = _dot_nt(lhs[:, i * T:(i + 1) * T], pk[:, i * T:(i + 1) * T])
            acc = part if acc is None else acc + part
        return jnp.where(mem_mask(), acc, 0.0)

    def mem_read(u, mem, gate):
        r = _dot(mem, _pad_bf16(_phi(u["q"])))
        coef = gate / (r[GR:GP] + 1e-6)
        out = []
        for i in range(NT):
            ci = coef[:, i * T:(i + 1) * T]
            wins = [jnp.broadcast_to(ci[j:j + 1], (24, T)) for j in range(HG)]
            out.append(r[0:GR, i * T:(i + 1) * T] * _merge_heads(wins))
        return out

    def finish(accs, gate, mem_i, turn):
        dens = [accs[j][LROW[j]:LROW[j] + 1] for j in range(HG)]
        o = _merge_heads([_rotate(accs[j] * ((1.0 - gate[j:j + 1]) / dens[j]), -j * turn)
                          for j in range(HG)])
        return (o if mem_i is None else o + mem_i), dens

    def out_rows(s, c, idx):
        rows = pl.ds(c * OC, OC)
        cols = pl.ds(s * L if isinstance(s, int) else pl.multiple_of(s * L, L), L)
        a = _dot(wot_s[rows], ot_s[s].astype(BF16))
        tok = _iota((1, L), 1) + s * L
        y0, y1 = (jnp.concatenate([y_s[n, rows]] * NT, axis=1) for n in range(2))
        upd = jnp.where(tok == idx[0], y0, jnp.where(tok == idx[1], y1, 0.0))
        xn = jnp.concatenate([xn_s[s * NT + i, rows] for i in range(NT)], axis=1)
        res = (x_v[rows, cols].astype(F32) + a) + (xn.astype(F32) + upd)
        o_v[rows, cols] = res.astype(BF16)
        return res

    def gates():
        sg = jax.nn.sigmoid(beta_ref[...].astype(F32).reshape(1, H))
        for g in range(NG):
            pick = _iota((8, H), 1) == _iota((8, H), 0) + HG * g
            col = jnp.sum(jnp.where(pick, sg, 0.0), axis=1, keepdims=True)
            g_s[g] = jnp.broadcast_to(col, (8, T))

    def pick(n):
        if n == 0:
            st["r"] = jnp.concatenate([st["r", t] for t in range(S // T)], axis=1)
            st["idx"], st["val"] = [], []
        tok = _iota((1, S), 1)
        best = jnp.max(st["r"], axis=1, keepdims=True)
        i = jnp.clip(jnp.min(jnp.where(st["r"] == best, tok, S)), 0, S - 1)
        st["r"] = jnp.where(tok == i, -jnp.inf, st["r"])
        st["idx"].append(i)
        st["val"].append(best)

    def gather(n):
        i = st["idx"][n]
        hot = ((_iota((8, T), 1) == i % T) & (_iota((8, T), 0) == n)).astype(F32)
        row = _dot_nt(hot, xn_s[i // T])
        st["xs"] = row if n == 0 else st["xs"] + row

    def ffn_in(name, w_ref, c, kt):
        lo, hi = kt * T, min((kt + 1) * T, D)
        part = _dot(st["xs"][:, lo:hi], w_ref[lo:hi, c * FC:(c + 1) * FC])
        st[name] = part if kt == 0 else st[name] + part

    def ffn_act(c):
        g = st["g"]
        h = _rb(g * jax.nn.sigmoid(g) * st["u"])
        for n in range(2):
            for f in range(FC // T):
                h_s[n, c * (FC // T) + f] = jnp.broadcast_to(h[n:n + 1, f * T:(f + 1) * T], (8, T))

    def ffn_out(r):
        acc = [0.0, 0.0]
        for f in range(FF // T):
            w = wd_v[r * 16:(r + 1) * 16, f * T:(f + 1) * T].astype(F32)
            for n in range(2):
                acc[n] = acc[n] + w * jnp.concatenate([h_s[n, f]] * 2, axis=0)
        for n in range(2):
            y = jnp.sum(acc[n], axis=1, keepdims=True) * jax.nn.sigmoid(st["val"][n])
            y_s[n, r * 16:(r + 1) * 16] = jnp.broadcast_to(y, (16, T))
        st["y", r] = (acc[0][0:8] + acc[0][8:16]) + (acc[1][0:8] + acc[1][8:16])

    units, mems = {}, {}
    tiles = [(u, i, c) for u in range(NSEG * NG) for i in ORDER for c in range(i + 1)]
    tri = _iota((QB, T), 0) <= _iota((QB, T), 1) % QB
    quarter = _iota((QB, T), 1) // QB
    odd, high = quarter % 2 == 1, quarter >= 2
    slot, head_of_row = _iota((GP, T), 1) // QB, _iota((GP, T), 0) // DH
    rng = dict(lo=jnp.ones((1, T), F32), hi=jnp.ones((1, T), F32), o=jnp.zeros((8, T), F32))

    def do_project(u):
        units[u] = project(u // NG, u % NG)

    def do_mem_read(u):
        gate = jnp.concatenate([g_s[u % NG]] * NT, axis=1)
        units[u]["mem"] = mem_read(units[u], mems[u % NG], gate)

    def do_mem_update(u):
        delta = mem_delta(units[u])
        mems[u % NG] = delta if u < NG else mems[u % NG] + delta

    def scores(t):
        u, i, c = tiles[t]
        un = units[u]
        if c == 0:
            q = un["q"][:, i * T:(i + 1) * T] * QSCALE
            qr = _merge_heads([_rotate(q[V0[j]:V0[j] + 24], j) for j in range(HG)])
            un["qr"] = jnp.concatenate([qr, jnp.zeros((GP - GR, T), F32)], axis=0)
            un["qm"] = jnp.concatenate([_head_query(qr, j) for j in range(HG)], axis=1)
        k = un["kn"][c * T:(c + 1) * T]
        if c < i:
            extra = QB if c == i - 1 else 0
            p = jnp.exp2(_dot(un["kn"][c * T:(c + 1) * T + extra], un["qm"]))
            st["p", t] = [p[0:T, j * T:(j + 1) * T].astype(BF16) for j in range(HG)]
            if extra:
                st["p0"] = p[T:]
            return
        p0 = st.pop("p0") if "p0" in st else jnp.exp2(_dot(k[0:QB], un["qm"]))
        e = {}
        for b in (3, 2, 1):
            w = jnp.where(slot == (head_of_row + b) % 4, un["qr"], 0.0).astype(BF16)
            r = jnp.exp2(_dot(k[QB:(b + 1) * QB], w))
            for a in range(1, b + 1):
                blk = r[(a - 1) * QB:a * QB]
                e[a, b] = jnp.where(tri, blk, 0.0) if a == b else blk
        x13 = [jnp.where(high, e[1, 3], e[1, 1]), jnp.where(high, e[1, 1], e[1, 3])]
        x23 = [jnp.where(odd, e[2, 3], e[2, 2]), jnp.where(odd, e[2, 2], e[2, 3])]
        ps = []
        for j in range(HG):
            block = (quarter - j) % 4
            outer = x13[(j + 1) % 4 // 2]
            x1 = jnp.where(odd, e[1, 2], outer) if j % 2 else jnp.where(odd, outer, e[1, 2])
            ps.append(jnp.concatenate(
                [jnp.where(tri | (block > 0), p0[:, j * T:(j + 1) * T], 0.0),
                 jnp.where(block >= 1, x1, 0.0),
                 jnp.where(block >= 2, x23[j % 2], 0.0),
                 jnp.where(block >= 3, e[3, 3], 0.0)], axis=0).astype(BF16))
        st["p", t] = ps

    def values(t):
        u, i, c = tiles[t]
        un = units[u]
        ps = st.pop(("p", t))
        v = un["v"][:, c * T:(c + 1) * T]
        one = 1.0
        for a in st.pop("due", []):
            one = jnp.maximum(jnp.minimum(a, one), one)
        for j in range(HG):
            part = _dot(_head_values(v, j, one), ps[j])
            st["o", j] = part if c == 0 else st["o", j] + part
        if c == i:
            mem_i = un["mem"][i] if "mem" in un else None
            o, dens = finish([st["o", j] for j in range(HG)], g_s[u % NG], mem_i, 1)
            ot_s[u // NG, (u % NG) * GR:(u % NG + 1) * GR, i * T:(i + 1) * T] = o
            for l in dens:
                rng["lo"], rng["hi"] = jnp.minimum(rng["lo"], l), jnp.maximum(rng["hi"], l)

    def due(*keys):
        st.setdefault("due", []).append(st[keys])

    def do_out(s, c):
        peak = jnp.max(jnp.abs(out_rows(s, c, st["idx"])).reshape(OC // 8, 8, L), axis=0)
        for i in range(NT):
            rng["o"] = jnp.maximum(rng["o"], peak[:, i * T:(i + 1) * T])
        st["peak", s, c] = rng["o"]
        rows, cols = pl.ds(c * OC, OC), pl.ds(s * L, L)
        start(("o", s, c), o_v.at[rows, cols], o_hbm.at[rows, cols])

    fill = {}

    def at(step, fn, *args):
        fill.setdefault(step, []).append((fn, args))

    nu = NSEG * NG
    for u in range(nu):
        t0 = u * STEPS
        if u + 1 < nu:
            at(t0 + (3 if u else 5), do_project, u + 1)
        if u >= NG:
            at(t0, do_mem_read, u)
        if u < nu - NG:
            at(t0 + 9, do_mem_update, u)
    at(2, second_batch)
    at(2, wait, ("wb", 0), ("wb", 1), ("wb", 2), "beta", "wr")
    at(2, gates)
    step = 3 * STEPS + 7
    at(2 * STEPS + 1, wait, ("wc", 0), ("wc", 1), ("wc", 2))
    at(step, third_batch)
    at(step, wait, "xc")
    for c in range(1, 5):
        for n in range(3):
            at(max((T * c // GR - 1) * STEPS + 2, 2), transpose_w, n, c)
    for t in range(S // T):
        if t < NT:
            at(STEPS + 4 + t * 5, router, t)
            at(STEPS + 4 + t * 5, due, "r", t)
        else:
            at(step, layernorm, t)
            at(step, router, t)
            at(4 * STEPS + 7 + (t - NT) * 5, due, "r", t)
    for n in range(2):
        at((11 + n) * STEPS + 6, pick, n)
        at((13 + n) * STEPS + 6, gather, n)
    step = 16 * STEPS + 7
    at(step, wait, "wo", "g", "u", "d")
    for c in range(5):
        at(step + c * STEPS, transpose_w, 3, c)
    for c in range(FF // FC):
        for name, w in (("g", wg_v), ("u", wu_v)):
            for kt in range(5):
                at(step, ffn_in, name, w, c, kt)
                step += 1
        at(step - 1, ffn_act, c)
    step += 2
    for r in range(D // 16):
        at(step, ffn_out, r)
        at(step, due, "y", r)
        step += 1
    chunks = [(s, c) for s in range(NSEG - 1) for c in range(D // OC)]
    gap = (len(tiles) - step - 6) // (len(chunks) - 1)
    for n, (s, c) in enumerate(chunks[:-1]):
        at(step + 6 + n * gap, do_out, s, c)
        at(step + 8 + n * gap, due, "peak", s, c)

    for i in range(NT - 1):
        wait(("x", i))
        layernorm(i)
    wait(("x", NT - 1))
    w_cols("wb", T, 2 * T)
    wait(("wa", 1))
    layernorm(NT - 1)
    transpose_w(1, 0)
    wait(("wa", 0))
    transpose_w(0, 0)
    k0 = _dot(wt_s[0, GR:2 * GR], seg_xn(0))
    wait(("wa", 2))
    transpose_w(2, 0)
    units[0] = unit_of(_dot(wt_s[0, 0:GR], seg_xn(0)), k0, _dot(wt_s[0, 2 * GR:3 * GR], seg_xn(0)))
    for t in range(len(tiles) + LAG):
        for fn, args in fill.pop(t, []):
            fn(*args)
        if t < len(tiles):
            scores(t)
        if t == len(tiles):
            do_out(*chunks[-1])
        if t >= LAG:
            values(t - LAG)
    assert not fill
    for c in range(D // OC):
        do_out(NSEG - 1, c)
    written = [key for key in copies if key[0] == "o"]
    wait(*written[:-1])
    safe = (jnp.min(rng["lo"]) >= L_LO) & (jnp.max(rng["hi"]) <= L_HI) & (jnp.max(rng["o"]) <= O_HI)
    wait(written[-1])

    @pl.when(jnp.logical_not(safe))
    def _():
        m_s[...] = jnp.zeros(m_s.shape, F32)

        def unit(u, carry):
            s, g = u // NG, u % NG
            un = project(s, g)
            gate = g_s[g]
            mem = mem_read(un, m_s[g], jnp.concatenate([gate] * NT, axis=1))
            for i in range(NT):
                nk = (i + 1) * T
                q = un["q"][:, i * T:nk] * QSCALE
                keep = _iota((nk, T), 0) <= _iota((nk, T), 1) + i * T
                accs = []
                for j in range(HG):
                    sc = jnp.where(keep, _dot(un["kn"][0:nk], _head_query(q, j)), -jnp.inf)
                    p = jnp.exp2(sc - jnp.max(sc, axis=0, keepdims=True))
                    accs.append(_dot(_head_values(un["v"][:, 0:nk], j), p.astype(BF16)))
                o, _ = finish(accs, gate, mem[i], 0)
                ot_s[s, pl.ds(pl.multiple_of(g * GR, 8), GR), i * T:nk] = o
            m_s[g] += mem_delta(un)
            return carry

        lax.fori_loop(0, nu, unit, 0)

        def segment(s, carry):
            for c in range(D // OC):
                out_rows(s, c, st["idx"])
            return carry

        lax.fori_loop(0, NSEG, segment, 0)
        redo = pltpu.make_async_copy(o_v, o_hbm, sems.at[0])
        redo.start()
        redo.wait()


@jax.jit
def pallas_parallel_sum__memory_aug_infini_attn__moe_arch_mod__prompt_kernel(
    A_x: jax.Array,
    A_wq: jax.Array,
    A_wk: jax.Array,
    A_wv: jax.Array,
    A_wo: jax.Array,
    A_beta: jax.Array,
    B_x: jax.Array,
    B_w_r: jax.Array,
    B_w_gate: jax.Array,
    B_w_up: jax.Array,
    B_w_down: jax.Array,
):
    del B_x
    hbm = pl.BlockSpec(memory_space=pltpu.HBM)
    nsem = 20 + NSEG * (D // OC)
    out = pl.pallas_call(
        _kernel,
        out_shape=jax.ShapeDtypeStruct((D, S), BF16),
        in_specs=[hbm] * 10,
        out_specs=hbm,
        scratch_shapes=[
            pltpu.VMEM((H,), BF16),
            pltpu.VMEM((D,), BF16),
            pltpu.VMEM((D, S), BF16),
            pltpu.VMEM((4, D, D), BF16),
            pltpu.VMEM((D, FF), BF16),
            pltpu.VMEM((D, FF), BF16),
            pltpu.VMEM((D, FF), BF16),
            pltpu.VMEM((S // T, D, T), BF16),
            pltpu.VMEM((NG, 3 * GR, D), F32),
            pltpu.VMEM((D, D), F32),
            pltpu.VMEM((NSEG, D, L), F32),
            pltpu.VMEM((D, S), BF16),
            pltpu.VMEM((2, FF // T, 8, T), F32),
            pltpu.VMEM((2, D, T), F32),
            pltpu.VMEM((NG, 8, T), F32),
            pltpu.VMEM((NG, GP, GP), F32),
            pltpu.SemaphoreType.DMA((nsem,)),
        ],
        compiler_params=pltpu.CompilerParams(vmem_limit_bytes=100 * 1024 * 1024),
        name="infini_mod",
    )(A_x.reshape(S, D).T, A_wq, A_wk, A_wv, A_wo, A_beta, B_w_r, B_w_gate, B_w_up, B_w_down.T)
    return out.T.reshape(1, S, D)
```
